```python
import os as _os
_os.environ.setdefault("JAX_PLATFORMS", "cpu")
import jax
import jax.numpy as jnp

def _softmax(x, axis=-1):
    return jax.nn.softmax(x, axis=axis)
def _gelu(x):
    return jax.nn.gelu(x, approximate=True)
def _silu(x):
    return jax.nn.silu(x)
def _sigmoid(x):
    return jax.nn.sigmoid(x)
def _layernorm(x, axis=-1, eps=1e-5):
    m = jnp.mean(x, axis=axis, keepdims=True)
    v = jnp.var(x, axis=axis, keepdims=True)
    return (x - m) / jnp.sqrt(v + eps)
def _scatter_add(tgt, idx, src, axis=0):
    return tgt.at[idx].add(src)
def _segment_sum(src, seg, n):
    return jax.ops.segment_sum(src, seg, n)
class _Rng:
    def __init__(self, key):
        self._k = key
    def _next(self):
        self._k, sub = jax.random.split(self._k)
        return sub
    def normal(self, shape):
        return jax.random.normal(self._next(), shape, dtype=jnp.bfloat16)
    def randint(self, lo, hi, shape):
        return jax.random.randint(self._next(), shape, lo, hi, dtype=jnp.int32)
    def uniform(self, shape, lo=0.0, hi=1.0):
        return jax.random.uniform(self._next(), shape, jnp.bfloat16, lo, hi)
    def permutation(self, n):
        return jax.random.permutation(self._next(), n)


kernel_name = 'gated_mix__linear_attn_block__sliding_local_dilated__prompt'

def setup_inputs():
    _rng = _Rng(jax.random.key(int.from_bytes(__import__("os").urandom(4), "little")))
    _w = (lambda a: (lambda t: t.astype(jnp.bfloat16) if jnp.issubdtype(t.dtype, jnp.floating) else t)(jnp.asarray(a)))
    def _A_setup():
        B, S, D = 1, 2048, 512
        return {
            "x": _w((lambda *s: _rng.normal(s) * 0.05)(B, S, D)),
            "wqkv": _w((lambda *s: _rng.normal(s) * 1.6)(D, 3 * D)),
            "wo": _w((lambda *s: _rng.normal(s) * 0.8)(D, D)),
        }
    _A_in = _A_setup()

    def _B_setup():
        B, S, D = 1, 2048, 512
        return {
            "x": _w((lambda *s: _rng.normal(s) * 0.05)(B, S, D)),
            "wqkv": _w((lambda *s: _rng.normal(s) * 0.8)(D, 3 * D)),
            "wo": _w((lambda *s: _rng.normal(s) * 0.05)(D, D)),
        }
    _B_in = _B_setup()

    return {
        "A_x": _A_in["x"],
        "A_wqkv": _A_in["wqkv"],
        "A_wo": _A_in["wo"],
        "B_x": _B_in["x"],
        "B_wqkv": _B_in["wqkv"],
        "B_wo": _B_in["wo"],
        "gate_w": _w((lambda *s: _rng.normal(s) * 0.05)(512) * 16.0),
    }

def reference(A_x, A_wqkv, A_wo, B_x, B_wqkv, B_wo, gate_w):
    def _A_ref(x, wqkv, wo):
        B, S, D = x.shape
        H = 32; Dh = D // H
        qkv = (lambda x, *d: x.transpose(*d))((x @ wqkv).reshape(B, S, 3, H, Dh), 2, 0, 3, 1, 4)
        q, k, v = qkv[0], qkv[1], qkv[2]
        phi = lambda t: jnp.where(t > 0, t + 1, jnp.exp(t)) + 1e-6
        pq, pk = phi(q), phi(k)
        kv = jnp.einsum("bhsd,bhse->bhde", pk, v)
        z = jnp.einsum("bhsd->bhd", pk)
        num = jnp.einsum("bhqd,bhde->bhqe", pq, kv)
        den = jnp.einsum("bhqd,bhd->bhq", pq, z)[..., None] + 1e-6
        o = num / den
        return (lambda x, *d: x.transpose(*d))(o, 0, 2, 1, 3).reshape(B, S, D) @ wo

    def _B_ref(x, wqkv, wo):
        B, S, D = x.shape
        H = 32; Dh = D // H
        W, dil = 8, 2
        qkv = (lambda x, *d: x.transpose(*d))((x @ wqkv).reshape(B, S, 3, H, Dh), 2, 0, 3, 1, 4)
        q, k, v = qkv[0], qkv[1], qkv[2]
        scale = Dh ** -0.5
        pos = jnp.arange(S)
        off = jnp.arange(W) * dil
        idx = pos[:, None] - off[None, :]
        mask = idx >= 0
        idx_c = jnp.where(mask, idx, 0).reshape(-1)
        kg = k[:, :, idx_c, :].reshape(B, H, S, W, Dh)
        vg = v[:, :, idx_c, :].reshape(B, H, S, W, Dh)
        logits = jnp.einsum("bhsd,bhswd->bhsw", q, kg) * scale
        logits = jnp.where(mask[None, None, :, :], logits, -1e9)
        attn = _softmax(logits, axis=-1)
        o = jnp.einsum("bhsw,bhswd->bhsd", attn, vg)
        return (lambda x, *d: x.transpose(*d))(o, 0, 2, 1, 3).reshape(B, S, D) @ wo

    x = A_x
    g = _sigmoid((x * gate_w).sum(-1, keepdims=True))
    a = _A_ref(x, A_wqkv, A_wo)
    b = _B_ref(x, B_wqkv, B_wo)
    return g * a + (1 - g) * b
```

```python
import functools
import jax
import jax.numpy as jnp
from jax import lax
import jax.experimental.pallas as pl
import jax.experimental.pallas.tpu as pltpu

S, D, H, DH, W, DIL = 2048, 512, 32, 16, 8, 2
T = 256
NT = S // T
R = 8
HALO = 16
ST = 20
SWAPS = [(1, 4), (1, 0), (1, 5), (1, 1), (0, 3), (0, 6), (0, 2)]
DD = [((d >> 1) & 1) * 8 + ((d >> 2) & 1) * 4 + ((d >> 3) & 1) * 2 + (d & 1) for d in range(16)]
F32 = jnp.float32
BF16 = jnp.bfloat16
U32 = jnp.uint32
QSCALE = (DH ** -0.5) * 1.4426950408889634
TOKROWS = 128
TAILCYC = 768
PROFILE = False
SCHED = [
    (['x0', 'wk'], ['x1', 'x2', 'x3'], ['rk', 'a0', 'b0']),
    (['x1', 'x2', 'x3'], ['x4', 'x5', 'wq', 'wb0', 'x6', 'x7', 'wb1'], ['a1', 'a2', 'b1', 'a3', 'b2']),
    (['x4', 'x5', 'wq', 'wb0'], ['wb2', 'wob', 'wv', 'woa'], ['a4', 'pq', 'b3', 'a5', 'p0', 'b4']),
    (['x6', 'x7', 'wb1', 'wb2', 'wob', 'wv', 'woa'], [], ['a6', 'p1', 'b5', 'a7', 'p2', 'b6', 'po', 'b7']),
]
MIDPOS = (2, 6)


def _scope(name):
    import contextlib
    return jax.named_scope(name) if PROFILE else contextlib.nullcontext()


def _phi(t):
    return jnp.where(t > 0, t + 1.0, jnp.exp(t)) + 1e-6


def _recip(x):
    r = pl.reciprocal(x, approx=True)
    return r * (2.0 - x * r)


def _lane_perm(chunks):
    lane = lax.broadcasted_iota(jnp.int32, chunks[0].shape, 1)
    chunks = list(chunks)
    for cb, j in SWAPS:
        bit = ((lane >> j) & 1) == 1
        out = list(chunks)
        for c in range(4):
            if (c >> cb) & 1 == 0:
                a = chunks[c]
                b = chunks[c | (1 << cb)]
                out[c] = jnp.where(bit, pltpu.roll(b, 1 << j, 1), a)
                out[c | (1 << cb)] = jnp.where(bit, b, pltpu.roll(a, 128 - (1 << j), 1))
        chunks = out
    return chunks


def _group_sum(p):
    p = p + pltpu.roll(p, 32, 1)
    p = p + pltpu.roll(p, 64, 1)
    return p


def _cs(c):
    return slice(c * 128, (c + 1) * 128)


def _pk(x):
    return pltpu.bitcast(x, U32)


def _up(u):
    return pltpu.bitcast(u, BF16)


def kernel(x_hbm, wa_hbm, woa_hbm, wb_hbm, wob_hbm, gw_ref, o_hbm,
           x_v, wa_v, woa_v, wb_v, wob_v, o_v,
           xu, wku, wc0, wc1, wc2, wc3, w2a, w2b, kv_ref, g_ref, z_ref, tmp_ref, tmp2_ref, ut0, ut1, gate_ref, pk_ref,
           qq0, qq1, k0, k1, v0, v1, lhs0, lhs1,
           sem_x, sem_w, sem_o, sem_z):
    qq = (qq0, qq1); kb = (k0, k1); vb = (v0, v1); lhs = (lhs0, lhs1)
    TH = T // 2
    wcat = (wc0, wc1, wc2, wc3)

    def cp_o(i):
        r = i * T if isinstance(i, int) else pl.multiple_of(i * T, T)
        return pltpu.make_async_copy(o_v.at[pl.ds(r, T), :], o_hbm.at[0, pl.ds(r, T), :], sem_o.at[i])

    cps = {}
    for i in range(NT):
        cps['x%d' % i] = pltpu.make_async_copy(x_hbm.at[0, pl.ds(i * T, T), :], x_v.at[pl.ds(i * T, T), :], sem_x.at[i])
    cps['wk'] = pltpu.make_async_copy(wa_hbm.at[:, 512:1024], wa_v.at[:, 512:1024], sem_w.at[0])
    cps['wq'] = pltpu.make_async_copy(wa_hbm.at[:, 0:512], wa_v.at[:, 0:512], sem_w.at[1])
    for m in range(3):
        cps['wb%d' % m] = pltpu.make_async_copy(wb_hbm.at[:, m * 512:(m + 1) * 512], wb_v.at[:, m * 512:(m + 1) * 512], sem_w.at[2 + m])
    cps['wob'] = pltpu.make_async_copy(wob_hbm, wob_v, sem_w.at[5])
    cps['wv'] = pltpu.make_async_copy(wa_hbm.at[:, 1024:1536], wa_v.at[:, 1024:1536], sem_w.at[6])
    cps['woa'] = pltpu.make_async_copy(woa_hbm, woa_v, sem_w.at[7])

    for n in SCHED[0][0]:
        cps[n].start()
    dz = pl.semaphore_read(sem_z)
    tok_row = pl.multiple_of(T + 8 * dz, 8)

    xtok_row = pl.multiple_of(S // 2 + 8 * dz, 8)

    dz8 = pl.multiple_of(8 * dz, 8)

    def deadline(ref):
        val = ref[pl.ds(dz8, 8), 0:128]
        if val.dtype != U32:
            val = pltpu.bitcast(val, U32)
        xu[pl.ds(xtok_row, 8), 0:128] = val

    def put_padded(tref, c, t, h0=0):
        for h in range(t.shape[0] // 16):
            tref[c, ST * (h0 + h):ST * (h0 + h) + 16, :] = t[16 * h:16 * h + 16, :]

    def gather_perm(tref, c):
        return jnp.concatenate([tref[c, pl.ds(DD[d], 32, stride=ST), :] for d in range(16)], axis=0)

    def row_perm_to(tref, dst_ref):
        for c in range(4):
            dst_ref[:, _cs(c)] = _pk(gather_perm(tref, c).astype(BF16))

    def prep_mat(uref, src_ref, off, m):
        for c in range(2):
            put_padded(uref, c, _pk(src_ref[c * 256:(c + 1) * 256, off:off + 512]).T)
        for c in range(2):
            wcat[m][c * 128:(c + 1) * 128, :] = gather_perm(uref, c).T

    def prep_wob(tref):
        for c in range(4):
            put_padded(tref, c, wob_v[:, _cs(c)].astype(F32))
        row_perm_to(tref, w2b)

    gw = gw_ref[...].astype(F32).reshape(1, D)

    def p1a(i):
        r0 = i * T
        xt = x_v[r0:r0 + T, :]
        xu[i * TH:(i + 1) * TH, :] = _pk(xt)
        gl = jnp.sum(xt.astype(F32) * gw, axis=-1, keepdims=True)
        gt = jnp.broadcast_to(jax.nn.sigmoid(gl), (T, 128))
        gate_ref[r0:r0 + T, :] = gt
        k = jnp.dot(_up(xu[i * TH:(i + 1) * TH, :]), _up(wku[...]), preferred_element_type=F32)
        pk = _phi(k)
        zs = pk.reshape(T // 8, 8, D).sum(axis=0)
        pk_ref[i * TH:(i + 1) * TH, :] = _pk(pk.astype(BF16))
        if i == 0:
            z_ref[...] = zs
        else:
            z_ref[...] += zs
        deadline(gate_ref)

    def p1b(i):
        gg = lax.dot_general(_up(pk_ref[i * TH:(i + 1) * TH, :]), _up(xu[i * TH:(i + 1) * TH, :]),
                             (((0,), (0,)), ((), ())), preferred_element_type=F32)
        if i == 0:
            g_ref[...] = gg
        else:
            g_ref[...] += gg

    def s1_pieces(h0, p):
        def piece(n):
            def f():
                xt = _up(xu[pl.ds(h0, TH), :])
                m, c = n // 4, n % 4
                res = jnp.dot(xt, _up(wcat[m][:, _cs(c)]), preferred_element_type=F32)
                if m == 0:
                    qq[p][0:T, _cs(c)] = res
                elif m == 1:
                    qq[p][0:T, _cs(4 + c)] = res * QSCALE
                else:
                    dst = kb[p] if m == 2 else vb[p]
                    dst[c, HALO:HALO + T, :] = res
                return [res[r - 8:r, :] for r in range(TOKROWS, T + 1, TOKROWS)]
            return (T, f)
        return [piece(n) for n in range(16)]

    def s3_pieces(r0, p, lo=0, hi=T):
        n_r = hi - lo

        def piece(n):
            def f():
                res = (jnp.dot(_up(lhs[p][lo // 2:hi // 2, 0:512]), _up(w2a[:, _cs(n)]), preferred_element_type=F32)
                       + jnp.dot(_up(lhs[p][lo // 2:hi // 2, 512:1024]), _up(w2b[:, _cs(n)]), preferred_element_type=F32))
                o_v[pl.ds(r0 + lo, n_r), _cs(n)] = res.astype(BF16)
                return [res[r - 8:r, :] for r in range(TOKROWS, n_r + 1, TOKROWS)]
            return (2 * n_r, f)
        return [piece(n) for n in range(4)]

    def halo(p):
        for c in range(4):
            kb[p][c, 0:HALO, :] = kb[1 - p][c, T:T + HALO, :]
            vb[p][c, 0:HALO, :] = vb[1 - p][c, T:T + HALO, :]

    def s2_pieces(r0, p, first):
        def piece(rs):
            def f():
                zrow = [z_ref[0:1, _cs(c)] for c in range(4)]
                g = gate_ref[pl.ds(r0 + rs, R), :]
                pq = [_phi(qq[p][rs:rs + R, _cs(c)]) for c in range(4)]
                t = pq[0] * zrow[0] + pq[1] * zrow[1] + pq[2] * zrow[2] + pq[3] * zrow[3]
                den = _group_sum(t) + 1e-6
                sa = g * _recip(den)
                outs = [pq[c] * sa for c in range(4)]
                q = [qq[p][rs:rs + R, _cs(4 + c)] for c in range(4)]
                ls = []
                for w in range(W):
                    st = HALO + rs - DIL * w
                    pp = q[0] * kb[p][0, st:st + R, :]
                    for c in range(1, 4):
                        pp = pp + q[c] * kb[p][c, st:st + R, :]
                    pp = _group_sum(pp)
                    if first and rs < DIL * w:
                        rowi = rs + lax.broadcasted_iota(jnp.int32, (R, 128), 0)
                        pp = jnp.where(rowi >= DIL * w, pp, -1e9)
                    ls.append(pp)
                m = ls[0]
                for w in range(1, W):
                    m = jnp.maximum(m, ls[w])
                es = [jnp.exp2(l - m) for l in ls]
                ssum = es[0]
                for w in range(1, W):
                    ssum = ssum + es[w]
                sb = (1.0 - g) * _recip(ssum)
                for c in range(4):
                    o = es[0] * vb[p][c, HALO + rs:HALO + rs + R, :]
                    for w in range(1, W):
                        st = HALO + rs - DIL * w
                        o = o + es[w] * vb[p][c, st:st + R, :]
                    outs.append(o * sb)
                return outs
            return f

        def pair(rs):
            fa, fb = piece(rs), piece(rs + 8)
            state = {}

            def first_():
                state['a'] = fa()

            def second_():
                b = fb()
                for c in range(8):
                    lhs[p][rs // 2:rs // 2 + 8, _cs(c)] = _pk(jnp.concatenate([state['a'][c], b[c]], axis=0).astype(BF16))
            return [first_, second_]

        out = []
        for rs in range(0, T, 16):
            out += pair(rs)
        return out

    def emit(mx, vp, p2, tailcyc):
        total = sum(c for c, _ in mx)
        span = max(total - tailcyc, 1)
        nv = len(vp)
        cyc = 0
        vp[0]()
        done = 1
        for c, f in mx:
            toks = f()
            for ti, tok in enumerate(toks):
                now = cyc + c * (ti + 1) / len(toks)
                upto = min(nv, 1 + int((nv - 1) * now / span + 0.5))
                if upto > done:
                    qq[p2][pl.ds(tok_row, 8), 0:128] = tok
                    for g_ in vp[done:upto]:
                        g_()
                    done = upto
            cyc += c
        for g_ in vp[done:]:
            g_()

    def step(h_s1, r_s2, r_s3, p2, extra=None, tailcyc=TAILCYC, first=False):
        a = s3_pieces(r_s3, 1 - p2) if r_s3 is not None else []
        if h_s1 is not None:
            halo(1 - p2)
            b = s1_pieces(h_s1, 1 - p2)
        else:
            b = []
        mx = a + b
        if extra is not None:
            mx = mx[:MIDPOS[0]] + [extra[0]] + mx[MIDPOS[0]:MIDPOS[1]] + [extra[1]] + mx[MIDPOS[1]:]
        emit(mx, s2_pieces(r_s2, p2, first), p2, tailcyc)

    def mid_pieces():
        row = lax.broadcasted_iota(jnp.int32, (128, 128), 0)
        col = lax.broadcasted_iota(jnp.int32, (128, 128), 1)
        bd = (row // 16) == (col // 16)

        def f1():
            for c in range(4):
                ghi = g_ref[_cs(c), :].astype(BF16)
                kv = jnp.dot(ghi, wa_v[:, 1024 + c * 128: 1024 + (c + 1) * 128], preferred_element_type=F32)
                kv_ref[c] = _pk(jnp.where(bd, kv, 0.0).astype(BF16))
            return []

        def f2():
            for c in range(4):
                mm = jnp.dot(_up(kv_ref[c]), woa_v[_cs(c), :], preferred_element_type=F32)
                for c2 in range(4):
                    put_padded(tmp_ref, c2, mm[:, _cs(c2)], h0=8 * c)
            row_perm_to(tmp_ref, w2a)
            return []
        return [(512, f1), (512, f2)]

    def do_work(wk):
        if wk == 'rk':
            wku[...] = _pk(wa_v[:, 512:1024])
        elif wk[0] == 'a':
            p1a(int(wk[1:]))
        elif wk[0] == 'b':
            p1b(int(wk[1:]))
        elif wk == 'pq':
            prep_mat(ut0, wa_v, 0, 0)
            deadline(wcat[0])
        elif wk == 'po':
            prep_wob(tmp2_ref)
            deadline(w2b)
        elif wk[0] == 'p':
            m = int(wk[1:])
            prep_mat(ut1 if m % 2 == 0 else ut0, wb_v, m * 512, m + 1)
            deadline(wcat[m + 1])

    for si, (waits, issues, work) in enumerate(SCHED):
        with _scope("w%d" % si):
            for n in waits:
                cps[n].wait()
            for n in issues:
                cps[n].start()
        if si < len(SCHED) - 1:
            with _scope("seg%d" % si):
                for wk in work:
                    do_work(wk)
    with _scope("seg_last"):
        for wk in SCHED[-1][2]:
            do_work(wk)
        z = jnp.sum(z_ref[...], axis=0, keepdims=True)
        z = jnp.broadcast_to(z, (8, D))
        zc = _lane_perm([z[:, _cs(c)] for c in range(4)])
        for c in range(4):
            z_ref[:, _cs(c)] = zc[c]
            kb[0][c, 0:HALO, :] = jnp.zeros((HALO, 128), F32)
            vb[0][c, 0:HALO, :] = jnp.zeros((HALO, 128), F32)
        for _, f in s1_pieces(0, 0):
            f()
        step(TH, 0, None, 0, extra=mid_pieces(), first=True)

    def pair_body(j, carry):
        i1 = 2 * j + 1
        r1 = pl.multiple_of(i1 * T, T)
        rm = pl.multiple_of(r1 - T, T)
        step(pl.multiple_of((i1 + 1) * TH, TH), r1, rm, 1)
        cp_o(i1 - 1).start()
        step(pl.multiple_of((i1 + 2) * TH, TH), pl.multiple_of(r1 + T, T), r1, 0)
        cp_o(i1).start()
        return carry

    with _scope("loop"):
        lax.fori_loop(0, (NT - 2) // 2, pair_body, 0)
    with _scope("tail"):
        rl = (NT - 1) * T
        vp = s2_pieces(rl, 1, False)
        nh = len(vp) // 2
        emit(s3_pieces((NT - 2) * T, 0), vp[:nh], 1, 512)
        cp_o(NT - 2).start()
        emit(s3_pieces(rl, 1, 0, T // 2), vp[nh:], 1, 256)
        cph = pltpu.make_async_copy(o_v.at[pl.ds(rl, T // 2), :], o_hbm.at[0, pl.ds(rl, T // 2), :], sem_o.at[NT])
        cph.start()
        for _, f in s3_pieces(rl, 1, T // 2, T):
            f()
        cpl = pltpu.make_async_copy(o_v.at[pl.ds(rl + T // 2, T // 2), :], o_hbm.at[0, pl.ds(rl + T // 2, T // 2), :], sem_o.at[NT - 1])
        cpl.start()
    with _scope("wend"):
        for i in range(NT - 1):
            cp_o(i).wait()
        cph.wait()
        cpl.wait()


@jax.jit
def pallas_gated_mix__linear_attn_block__sliding_local_dilated__prompt_kernel(A_x, A_wqkv, A_wo, B_x, B_wqkv, B_wo, gate_w):
    anyspec = pl.BlockSpec(memory_space=pl.ANY)
    out = pl.pallas_call(
        kernel,
        grid=(1,),
        in_specs=[anyspec] * 5 + [pl.BlockSpec((D,), lambda i: (0,))],
        out_specs=anyspec,
        out_shape=jax.ShapeDtypeStruct((1, S, D), BF16),
        scratch_shapes=[
            pltpu.VMEM((S, D), BF16),
            pltpu.VMEM((D, 1536), BF16),
            pltpu.VMEM((D, D), BF16),
            pltpu.VMEM((D, 1536), BF16),
            pltpu.VMEM((D, D), BF16),
            pltpu.VMEM((S, D), BF16),
            pltpu.VMEM((S // 2 + 8, D), U32),
            pltpu.VMEM((D // 2, D), U32),
            pltpu.VMEM((D // 2, D), U32), pltpu.VMEM((D // 2, D), U32), pltpu.VMEM((D // 2, D), U32), pltpu.VMEM((D // 2, D), U32),
            pltpu.VMEM((D // 2, D), U32), pltpu.VMEM((D // 2, D), U32),
            pltpu.VMEM((4, 64, 128), U32),
            pltpu.VMEM((D, D), F32),
            pltpu.VMEM((8, D), F32),
            pltpu.VMEM((4, 32 * ST, 128), F32),
            pltpu.VMEM((4, 32 * ST, 128), F32),
            pltpu.VMEM((2, 32 * ST, 128), U32),
            pltpu.VMEM((2, 32 * ST, 128), U32),
            pltpu.VMEM((S, 128), F32),
            pltpu.VMEM((S // 2, D), U32),
            pltpu.VMEM((T + 8, 2 * D), F32), pltpu.VMEM((T + 8, 2 * D), F32),
            pltpu.VMEM((4, HALO + T, 128), F32), pltpu.VMEM((4, HALO + T, 128), F32),
            pltpu.VMEM((4, HALO + T, 128), F32), pltpu.VMEM((4, HALO + T, 128), F32),
            pltpu.VMEM((T // 2, 1024), U32), pltpu.VMEM((T // 2, 1024), U32),
            pltpu.SemaphoreType.DMA((NT,)),
            pltpu.SemaphoreType.DMA((8,)),
            pltpu.SemaphoreType.DMA((NT + 1,)),
            pltpu.SemaphoreType.REGULAR,
        ],
        compiler_params=pltpu.CompilerParams(vmem_limit_bytes=100 * 1024 * 1024),
    )(A_x, A_wqkv, A_wo, B_wqkv, B_wo, gate_w)
    return out
```

```python
import functools
import jax
import jax.numpy as jnp
from jax import lax
import jax.experimental.pallas as pl
import jax.experimental.pallas.tpu as pltpu

S, D, H, DH, W, DIL = 2048, 512, 32, 16, 8, 2
T = 256
NT = S // T
R = 8
HALO = 16
ST = 20
SWAPS = [(1, 4), (1, 0), (1, 5), (1, 1), (0, 3), (0, 6), (0, 2)]
DD = [((d >> 1) & 1) * 8 + ((d >> 2) & 1) * 4 + ((d >> 3) & 1) * 2 + (d & 1) for d in range(16)]
F32 = jnp.float32
BF16 = jnp.bfloat16
U32 = jnp.uint32
LOG2E = 1.4426950408889634
QSCALE = (DH ** -0.5) * LOG2E
TOKROWS = 64
SKEW = 1
TAILCYC = 768
PROFILE = False
SCHED = [
    (['gw', 'x0', 'wk'], ['x1', 'x2', 'x3'], ['rk0', 'A0']),
    (['wk2'], ['x4', 'x5'], ['rk1', 'B0', 'b0']),
    (['x1', 'x2', 'x3'], ['wq', 'wb0', 'x6', 'x7', 'wb1', 'wb2'], ['a1', 'a2', 'b1', 'a3', 'b2']),
    (['x4', 'x5', 'wq', 'wb0'], ['wob', 'wv', 'woa'], ['a4', 'pq', 'b3', 'a5', 'p0', 'b4']),
    (['x6', 'x7', 'wb1', 'wb2', 'wob', 'wv', 'woa'], [], ['a6', 'p1', 'b5', 'p2', 'a7']),
]
MIDPOS = (3, 8)
NA0 = 27
NH7 = 66
TC7 = 0


def _scope(name):
    import contextlib
    return jax.named_scope(name) if PROFILE else contextlib.nullcontext()


def _phi(t):
    return jnp.where(t > 0, t + 1.0, jnp.exp(t)) + 1e-6


def _recip(x):
    r = pl.reciprocal(x, approx=True)
    return r * (2.0 - x * r)


def _lane_perm(chunks):
    lane = lax.broadcasted_iota(jnp.int32, chunks[0].shape, 1)
    chunks = list(chunks)
    for cb, j in SWAPS:
        bit = ((lane >> j) & 1) == 1
        out = list(chunks)
        for c in range(4):
            if (c >> cb) & 1 == 0:
                a = chunks[c]
                b = chunks[c | (1 << cb)]
                out[c] = jnp.where(bit, pltpu.roll(b, 1 << j, 1), a)
                out[c | (1 << cb)] = jnp.where(bit, b, pltpu.roll(a, 128 - (1 << j), 1))
        chunks = out
    return chunks


def _group_sum(p):
    p = p + pltpu.roll(p, 32, 1)
    p = p + pltpu.roll(p, 64, 1)
    return p


def _cs(c):
    return slice(c * 128, (c + 1) * 128)


def _pk(x):
    return pltpu.bitcast(x, U32)


def _up(u):
    return pltpu.bitcast(u, BF16)


def kernel(x_hbm, wa_hbm, woa_hbm, wb_hbm, wob_hbm, gw_hbm, zero_hbm, o_hbm,
           zero_s, gw_ref, x_v, wa_v, woa_v, wb_v, wob_v, o_v,
           xu, wku, wc0, wc1, wc2, wc3, w2a, w2b, kv_ref, g_ref, z_ref, tmp_ref, tmp2_ref, ut0, ut1, gate_ref, pk_ref,
           qq0, qq1, k0, k1, v0, v1, lhs0, lhs1,
           cb, sem_x, sem_w, sem_o):
    qq = (qq0, qq1); kb = (k0, k1); vb = (v0, v1); lhs = (lhs0, lhs1)
    TH = T // 2
    wcat = (wc0, wc1, wc2, wc3)

    def cp_o(i):
        r = i * T if isinstance(i, int) else pl.multiple_of(i * T, T)
        return pltpu.make_async_copy(o_v.at[pl.ds(r, T), :], o_hbm.at[0, pl.ds(r, T), :], sem_o.at[i])

    cps = {}
    for i in range(NT):
        cps['x%d' % i] = pltpu.make_async_copy(x_hbm.at[0, pl.ds(i * T, T), :], x_v.at[pl.ds(i * T, T), :], sem_x.at[i])
    cps['wk'] = pltpu.make_async_copy(wa_hbm.at[:, 512:768], wa_v.at[:, 512:768], sem_w.at[0])
    cps['wk2'] = pltpu.make_async_copy(wa_hbm.at[:, 768:1024], wa_v.at[:, 768:1024], sem_w.at[9])
    cps['wq'] = pltpu.make_async_copy(wa_hbm.at[:, 0:512], wa_v.at[:, 0:512], sem_w.at[1])
    for m in range(3):
        cps['wb%d' % m] = pltpu.make_async_copy(wb_hbm.at[:, m * 512:(m + 1) * 512], wb_v.at[:, m * 512:(m + 1) * 512], sem_w.at[2 + m])
    cps['wob'] = pltpu.make_async_copy(wob_hbm, wob_v, sem_w.at[5])
    cps['wv'] = pltpu.make_async_copy(wa_hbm.at[:, 1024:1536], wa_v.at[:, 1024:1536], sem_w.at[6])
    cps['woa'] = pltpu.make_async_copy(woa_hbm, woa_v, sem_w.at[7])
    cps['gw'] = pltpu.make_async_copy(gw_hbm, gw_ref, sem_w.at[8])

    cpz = pltpu.make_async_copy(zero_hbm, zero_s, sem_w.at[10])
    cpz.start()
    for n in SCHED[0][0] + ['wk2']:
        cps[n].start()
    cpz.wait()
    dz = zero_s[0]
    tok_row = pl.multiple_of(40 + 8 * dz, 8)
    for ci, cv in enumerate([QSCALE, 0.0, 1.0, LOG2E, -3.0e38]):
        cb[8 * ci:8 * ci + 8, :] = jnp.full((8, 128), cv, F32)

    xtok_row = pl.multiple_of(S // 2 + 8 * dz, 8)

    dz8 = pl.multiple_of(8 * dz, 8)

    def deadline(ref):
        val = ref[pl.ds(dz8, 8), 0:128]
        if val.dtype != U32:
            val = pltpu.bitcast(val, U32)
        xu[pl.ds(xtok_row, 8), 0:128] = val

    def put_padded(tref, c, t, h0=0):
        for h in range(t.shape[0] // 16):
            tref[c, ST * (h0 + h):ST * (h0 + h) + 16, :] = t[16 * h:16 * h + 16, :]

    def gather_perm(tref, c):
        return jnp.concatenate([tref[c, pl.ds(DD[d], 32, stride=ST), :] for d in range(16)], axis=0)

    def row_perm_to(tref, dst_ref):
        for c in range(4):
            dst_ref[:, _cs(c)] = _pk(gather_perm(tref, c).astype(BF16))

    def prep_mat(uref, src_ref, off, m):
        for c in range(2):
            put_padded(uref, c, _pk(src_ref[c * 256:(c + 1) * 256, off:off + 512]).T)
        for c in range(2):
            wcat[m][c * 128:(c + 1) * 128, :] = gather_perm(uref, c).T

    def prep_wob(tref):
        for c in range(4):
            put_padded(tref, c, wob_v[:, _cs(c)].astype(F32))
        row_perm_to(tref, w2b)

    def p1a(i, part=None):
        r0 = i * T
        if part != 1:
            xt = x_v[r0:r0 + T, :]
            xu[i * TH:(i + 1) * TH, :] = _pk(xt)
            gw = gw_ref[...].astype(F32).reshape(1, D)
            gl = jnp.sum(xt.astype(F32) * gw, axis=-1, keepdims=True)
            gt = jnp.broadcast_to(jax.nn.sigmoid(gl), (T, 128))
            gate_ref[r0:r0 + T, :] = gt
        cols = slice(0, D) if part is None else slice(part * 256, (part + 1) * 256)
        nc = D if part is None else 256
        k = jnp.dot(_up(xu[i * TH:(i + 1) * TH, :]), _up(wku[:, cols]), preferred_element_type=F32)
        pk = _phi(k)
        zs = pk.reshape(T // 8, 8, nc).sum(axis=0)
        pk_ref[i * TH:(i + 1) * TH, cols] = _pk(pk.astype(BF16))
        if i == 0:
            z_ref[:, cols] = zs
        else:
            z_ref[:, cols] += zs
        if part is None:
            deadline(gate_ref)

    def p1b(i):
        gg = lax.dot_general(_up(pk_ref[i * TH:(i + 1) * TH, :]), _up(xu[i * TH:(i + 1) * TH, :]),
                             (((0,), (0,)), ((), ())), preferred_element_type=F32)
        if i == 0:
            g_ref[...] = gg
        else:
            g_ref[...] += gg
        return [gg[r - 8:r, c * 128:(c + 1) * 128] for c in range(4) for r in range(128, 513, 128)]

    def s1_pieces(h0, p, lo=0, hi=T):
        n_r = hi - lo

        def piece(n):
            def f():
                xt = _up(xu[pl.ds(h0 + lo // 2, n_r // 2), :])
                m, c = n // 4, n % 4
                res = jnp.dot(xt, _up(wcat[m][:, _cs(c)]), preferred_element_type=F32)
                if m == 0:
                    qq[p][lo:hi, _cs(c)] = res
                elif m == 1:
                    qq[p][lo:hi, _cs(4 + c)] = res
                else:
                    dst = kb[p] if m == 2 else vb[p]
                    dst[c, HALO + lo:HALO + hi, :] = res
                return [res[r - 8:r, :] for r in range(TOKROWS, n_r + 1, TOKROWS)]
            return (n_r, f)
        return [piece(n) for n in range(16)]

    def s3_pieces(r0, p, lo=0, hi=T):
        n_r = hi - lo

        def piece(n):
            def f():
                res1 = jnp.dot(_up(lhs[p][lo // 2:hi // 2, 0:512]), _up(w2a[:, _cs(n)]), preferred_element_type=F32)
                res = res1 + jnp.dot(_up(lhs[p][lo // 2:hi // 2, 512:1024]), _up(w2b[:, _cs(n)]), preferred_element_type=F32)
                o_v[pl.ds(r0 + lo, n_r), _cs(n)] = res.astype(BF16)
                return ([res1[r - 8:r, :] for r in range(TOKROWS, n_r + 1, TOKROWS)]
                        + [res[r - 8:r, :] for r in range(TOKROWS, n_r + 1, TOKROWS)])
            return (2 * n_r, f)
        return [piece(n) for n in range(4)]

    def halo(p):
        for c in range(4):
            kb[p][c, 0:HALO, :] = kb[1 - p][c, T:T + HALO, :]
            vb[p][c, 0:HALO, :] = vb[1 - p][c, T:T + HALO, :]

    def s2_pieces(r0, p, first):
        out = []
        for rs in range(0, T, R):
            st_ = {}

            def part_a(rs=rs, st_=st_):
                zrow = [z_ref[0:1, _cs(c)] for c in range(4)]
                g = gate_ref[pl.ds(r0 + rs, R), :]
                st_['g'] = g
                c0, c1, cl = cb[8:16, :], cb[16:24, :], cb[24:32, :]
                pq = []
                for c in range(4):
                    tq = qq[p][rs:rs + R, _cs(c)]
                    pq.append(jnp.where(tq > c0, tq + c1, jnp.exp2(tq * cl)) + 1e-6)
                t = pq[0] * zrow[0] + pq[1] * zrow[1] + pq[2] * zrow[2] + pq[3] * zrow[3]
                den = _group_sum(t) + 1e-6
                sa = g * _recip(den)
                put(rs, 0, [pq[c] * sa for c in range(4)])

            def part_qk(rs=rs, st_=st_):
                sc = cb[0:8, :]
                q = [qq[p][rs:rs + R, _cs(4 + c)] * sc for c in range(4)]
                ls = []
                for w in range(W):
                    st = HALO + rs - DIL * w
                    pp = q[0] * kb[p][0, st:st + R, :]
                    for c in range(1, 4):
                        pp = pp + q[c] * kb[p][c, st:st + R, :]
                    pp = _group_sum(pp)
                    if first and rs < DIL * w:
                        rowi = rs + lax.broadcasted_iota(jnp.int32, (R, 128), 0)
                        pp = jnp.where(rowi >= DIL * w, pp, -1e9)
                    ls.append(pp)
                m = ls[0]
                for w in range(1, W):
                    m = jnp.maximum(m, ls[w])
                st_['ls'] = ls
                st_['m'] = m

            def part_av(rs=rs, st_=st_):
                ls = st_['ls']
                m = jnp.maximum(st_['m'], cb[32:40, :])
                es = [jnp.exp2(l - m) for l in ls]
                ssum = es[0]
                for w in range(1, W):
                    ssum = ssum + es[w]
                sb = (1.0 - st_['g']) * _recip(ssum)
                outs = []
                for c in range(4):
                    o = es[0] * vb[p][c, HALO + rs:HALO + rs + R, :]
                    for w in range(1, W):
                        st = HALO + rs - DIL * w
                        o = o + es[w] * vb[p][c, st:st + R, :]
                    outs.append(o * sb)
                put(rs, 4, outs)

            out.append([('c', part_a), ('c', part_qk), ('c', part_av)])

        pend = {}

        def put(rs, c0, vals):
            key = (rs // 16, c0)
            if rs % 16 == 0:
                pend[key] = vals
            else:
                a_ = pend.pop(key)
                r2 = (rs - 8) // 2
                for c in range(4):
                    lhs[p][r2:r2 + 8, _cs(c0 + c)] = _pk(jnp.concatenate([a_[c], vals[c]], axis=0).astype(BF16))

        seq = []
        n = len(out)
        for i in range(n + SKEW):
            if i < n:
                seq.append(out[i][0])
                seq.append(out[i][1])
            if i - SKEW >= 0:
                seq.append(out[i - SKEW][2])
        return seq

    def token(p2, tgt, tok):
        cb[pl.ds(tok_row, 8), :] = tok

    def emit(mx, vp, p2, tailcyc, gate_at=None):
        total = sum(c for c, _ in mx)
        span = max(total - tailcyc, 1)
        nv = len(vp)
        cyc = 0
        vp[0][1]()
        done = 1
        for c, f in mx:
            toks = f()
            for ti, tok in enumerate(toks):
                now = cyc + c * (ti + 1) / len(toks)
                upto = min(nv, 1 + int((nv - 1) * now / span + 0.5))
                if gate_at is not None and now < gate_at[1]:
                    upto = min(upto, gate_at[0])
                if upto > done:
                    for tgt in sorted(set(t for t, _ in vp[done:upto])):
                        token(p2, tgt, tok)
                    for _, g_ in vp[done:upto]:
                        g_()
                    done = upto
            cyc += c
        for _, g_ in vp[done:]:
            g_()

    HT = T // 2

    def step(h_cur, h_next, r_s2, r_s3, p2, extra=None, tailcyc=TAILCYC, first=False):
        mx = s1_pieces(h_cur, p2, HT, T)
        gate_cyc = sum(c for c, _ in mx)
        if extra is not None:
            mx = mx + [(1024, lambda: p1b(6)), (1024, lambda: p1b(7))]
        if r_s3 is not None:
            mx = mx + s3_pieces(r_s3, 1 - p2)
        if h_next is not None:
            nxt = s1_pieces(h_next, 1 - p2, 0, HT)
            c0, f0 = nxt[0]

            def f0h():
                halo(1 - p2)
                return f0()
            nxt = [(c0, f0h)] + nxt[1:]
            if extra is not None:
                nxt = nxt[:MIDPOS[0]] + [extra[0]] + nxt[MIDPOS[0]:MIDPOS[1]] + [extra[1]] + nxt[MIDPOS[1]:]
            mx = mx + nxt
        vp = s2_pieces(r_s2, p2, first)
        ngate = 2 * (HT // R) + (HT // R - SKEW)
        emit(mx, vp, p2, tailcyc, gate_at=(ngate, gate_cyc))

    def mid_pieces():
        row = lax.broadcasted_iota(jnp.int32, (128, 128), 0)
        col = lax.broadcasted_iota(jnp.int32, (128, 128), 1)
        bd = (row // 16) == (col // 16)

        def f1():
            toks = []
            for c in range(4):
                ghi = g_ref[_cs(c), :].astype(BF16)
                kv = jnp.dot(ghi, wa_v[:, 1024 + c * 128: 1024 + (c + 1) * 128], preferred_element_type=F32)
                kv_ref[c] = _pk(jnp.where(bd, kv, 0.0).astype(BF16))
                toks += [kv[56:64, :], kv[120:128, :]]
            return toks

        def f2():
            toks = []
            for c in range(4):
                mm = jnp.dot(_up(kv_ref[c]), woa_v[_cs(c), :], preferred_element_type=F32)
                for c2 in range(4):
                    put_padded(tmp_ref, c2, mm[:, _cs(c2)], h0=8 * c)
                toks += [mm[56:64, 0:128], mm[120:128, 0:128]]
            row_perm_to(tmp_ref, w2a)
            return toks
        return [(512, f1), (512, f2)]

    def do_work(wk):
        if wk == 'rk0':
            wku[:, 0:256] = _pk(wa_v[:, 512:768])
        elif wk == 'rk1':
            wku[:, 256:512] = _pk(wa_v[:, 768:1024])
        elif wk == 'A0':
            p1a(0, 0)
        elif wk == 'B0':
            p1a(0, 1)
        elif wk[0] == 'a':
            p1a(int(wk[1:]))
        elif wk[0] == 'b':
            p1b(int(wk[1:]))
        elif wk == 'pq':
            prep_mat(ut0, wa_v, 0, 0)
            deadline(wcat[0])
        elif wk == 'po':
            prep_wob(tmp2_ref)
            deadline(w2b)
        elif wk[0] == 'p':
            m = int(wk[1:])
            prep_mat(ut1 if m % 2 == 0 else ut0, wb_v, m * 512, m + 1)
            deadline(wcat[m + 1])

    for si, (waits, issues, work) in enumerate(SCHED):
        with _scope("w%d" % si):
            for n in waits:
                cps[n].wait()
            for n in issues:
                cps[n].start()
        if si < len(SCHED) - 1:
            with _scope("seg%d" % si):
                for wk in work:
                    do_work(wk)
    with _scope("seg_last"):
        for wk in SCHED[-1][2]:
            do_work(wk)
        z = jnp.sum(z_ref[...], axis=0, keepdims=True)
        z = jnp.broadcast_to(z, (8, D))
        zc = _lane_perm([z[:, _cs(c)] for c in range(4)])
        for c in range(4):
            z_ref[:, _cs(c)] = zc[c]
            kb[0][c, 0:HALO, :] = jnp.zeros((HALO, 128), F32)
            vb[0][c, 0:HALO, :] = jnp.zeros((HALO, 128), F32)
        for pi, (_, f) in enumerate(s1_pieces(0, 0, 0, HT)):
            toks = f()
            if pi % 4 == 0:
                c = pi // 4
                tmp2_ref[c, pl.ds(pl.multiple_of(32 * ST + 8 * dz, 8), 8), :] = toks[0]
                put_padded(tmp2_ref, c, wob_v[:, _cs(c)].astype(F32))
                w2b[:, _cs(c)] = _pk(gather_perm(tmp2_ref, c).astype(BF16))
        step(0, TH, 0, None, 0, extra=mid_pieces(), first=True)

    def pair_body(j, carry):
        i1 = 2 * j + 1
        r1 = pl.multiple_of(i1 * T, T)
        rm = pl.multiple_of(r1 - T, T)
        h1 = pl.multiple_of(i1 * TH, TH)
        h2 = pl.multiple_of((i1 + 1) * TH, TH)
        h3 = pl.multiple_of((i1 + 2) * TH, TH)
        step(h1, h2, r1, rm, 1)
        cp_o(i1 - 1).start()
        step(h2, h3, pl.multiple_of(r1 + T, T), r1, 0)
        cp_o(i1).start()
        return carry

    with _scope("loop"):
        lax.fori_loop(0, (NT - 2) // 2, pair_body, 0)
    with _scope("tail"):
        rl = (NT - 1) * T
        step((NT - 1) * TH, None, rl, (NT - 2) * T, 1, tailcyc=TC7)
        cp_o(NT - 2).start()
        for _, f in s3_pieces(rl, 1, 0, HT):
            f()
        cph = pltpu.make_async_copy(o_v.at[pl.ds(rl, HT), :], o_hbm.at[0, pl.ds(rl, HT), :], sem_o.at[NT])
        cph.start()
        for _, f in s3_pieces(rl, 1, HT, T):
            f()
        cpl = pltpu.make_async_copy(o_v.at[pl.ds(rl + HT, HT), :], o_hbm.at[0, pl.ds(rl + HT, HT), :], sem_o.at[NT - 1])
        cpl.start()
    with _scope("wend"):
        for i in range(NT - 1):
            cp_o(i).wait()
        cph.wait()
        cpl.wait()


@jax.jit
def pallas_gated_mix__linear_attn_block__sliding_local_dilated__prompt_kernel(A_x, A_wqkv, A_wo, B_x, B_wqkv, B_wo, gate_w):
    anyspec = pl.BlockSpec(memory_space=pl.ANY)
    out = pl.pallas_call(
        kernel,
        grid=(1,),
        in_specs=[anyspec] * 7,
        out_specs=anyspec,
        out_shape=jax.ShapeDtypeStruct((1, S, D), BF16),
        scratch_shapes=[
            pltpu.SMEM((8,), jnp.int32),
            pltpu.VMEM((D,), BF16),
            pltpu.VMEM((S, D), BF16),
            pltpu.VMEM((D, 1536), BF16),
            pltpu.VMEM((D, D), BF16),
            pltpu.VMEM((D, 1536), BF16),
            pltpu.VMEM((D, D), BF16),
            pltpu.VMEM((S, D), BF16),
            pltpu.VMEM((S // 2 + 8, D), U32),
            pltpu.VMEM((D // 2, D), U32),
            pltpu.VMEM((D // 2, D), U32), pltpu.VMEM((D // 2, D), U32), pltpu.VMEM((D // 2, D), U32), pltpu.VMEM((D // 2, D), U32),
            pltpu.VMEM((D // 2, D), U32), pltpu.VMEM((D // 2, D), U32),
            pltpu.VMEM((4, 64, 128), U32),
            pltpu.VMEM((D, D), F32),
            pltpu.VMEM((8, D), F32),
            pltpu.VMEM((4, 32 * ST, 128), F32),
            pltpu.VMEM((4, 32 * ST + 8, 128), F32),
            pltpu.VMEM((2, 32 * ST, 128), U32),
            pltpu.VMEM((2, 32 * ST, 128), U32),
            pltpu.VMEM((S, 128), F32),
            pltpu.VMEM((S // 2, D), U32),
            pltpu.VMEM((T, 2 * D), F32), pltpu.VMEM((T, 2 * D), F32),
            pltpu.VMEM((4, HALO + T, 128), F32), pltpu.VMEM((4, HALO + T, 128), F32),
            pltpu.VMEM((4, HALO + T, 128), F32), pltpu.VMEM((4, HALO + T, 128), F32),
            pltpu.VMEM((T // 2, 1024), U32), pltpu.VMEM((T // 2, 1024), U32),
            pltpu.VMEM((48, 128), F32),
            pltpu.SemaphoreType.DMA((NT,)),
            pltpu.SemaphoreType.DMA((11,)),
            pltpu.SemaphoreType.DMA((NT + 1,)),
        ],
        compiler_params=pltpu.CompilerParams(vmem_limit_bytes=100 * 1024 * 1024),
    )(A_x, A_wqkv, A_wo, B_wqkv, B_wo, gate_w, jnp.zeros((8,), jnp.int32))
    return out
```

```python
import jax
import jax.numpy as jnp
from jax import lax
import jax.experimental.pallas as pl
import jax.experimental.pallas.tpu as pltpu

S, D, DH, W, DIL = 2048, 512, 16, 8, 2
T = 256
TH = T // 2
HT = T // 2
NT = S // T
R = 8
HALO = 16
ST = 20
SWAPS = [(1, 4), (1, 0), (1, 5), (1, 1), (0, 3), (0, 6), (0, 2)]
DD = [((d >> 1) & 1) * 8 + ((d >> 2) & 1) * 4 + ((d >> 3) & 1) * 2 + (d & 1) for d in range(16)]
F32, BF16, U32 = jnp.float32, jnp.bfloat16, jnp.uint32
LOG2E = 1.4426950408889634
QSCALE = (DH ** -0.5) * LOG2E
TOKROWS = 32
TAILCYC = 512
PATTERN = ((1, 0), (1, 1), (0, 0), (0, 1), (2, 0), (2, 1))
SCHED = [
    (['gw', 'x0', 'wk'], ['x1', 'x2', 'x3'], ['rk0', 'A0']),
    (['wk2'], ['x4', 'x5'], ['rk1', 'B0', 'b0']),
    (['x1', 'x2', 'x3'], ['wq', 'wb0', 'x6', 'x7', 'wb1', 'wb2'], ['a1', 'a2', 'b1', 'g', 'a3', 'g', 'b2']),
    (['x4', 'x5', 'wq', 'wb0'], ['wob', 'wv', 'woa'], ['pq', 'p0', 'a4', 'b3', 'd0', 'a5', 'g', 'd1', 'b4']),
    (['x6', 'x7', 'wb1', 'wb2', 'wob', 'wv', 'woa'], [], ['p1', 'p2', 'a6', 'b5', 'd2', 'a7', 'g']),
]


def _phi(t):
    return jnp.where(t > 0, t + 1.0, jnp.exp(t)) + 1e-6


def _recip(x):
    r = pl.reciprocal(x, approx=True)
    return r * (2.0 - x * r)


def _lane_perm(chunks):
    lane = lax.broadcasted_iota(jnp.int32, chunks[0].shape, 1)
    chunks = list(chunks)
    for cbit, j in SWAPS:
        bit = ((lane >> j) & 1) == 1
        out = list(chunks)
        for c in range(4):
            if (c >> cbit) & 1 == 0:
                a = chunks[c]
                b = chunks[c | (1 << cbit)]
                out[c] = jnp.where(bit, pltpu.roll(b, 1 << j, 1), a)
                out[c | (1 << cbit)] = jnp.where(bit, b, pltpu.roll(a, 128 - (1 << j), 1))
        chunks = out
    return chunks


def _group_sum(p):
    p = p + pltpu.roll(p, 32, 1)
    return p + pltpu.roll(p, 64, 1)


def _cs(c):
    return slice(c * 128, (c + 1) * 128)


def _pk(x):
    return pltpu.bitcast(x, U32)


def _up(u):
    return pltpu.bitcast(u, BF16)


def _kernel(x_hbm, wa_hbm, woa_hbm, wb_hbm, wob_hbm, gw_hbm, zero_hbm, o_hbm,
            zero_s, gw_ref, x_v, wa_v, woa_v, wb_v, wob_v, o_v,
            xu, wku, wc0, wc1, wc2, wc3, w2a, w2b, kv_ref, g_ref, z_ref, tmp_ref, tmp2_ref, ut0, ut1,
            gate_ref, pk_ref, qq0, qq1, k0, k1, v0, v1, lhs0, lhs1, cb, sem_x, sem_w, sem_o):
    qq, kb, vb, lhs = (qq0, qq1), (k0, k1), (v0, v1), (lhs0, lhs1)
    wcat = (wc0, wc1, wc2, wc3)

    def cp_o(i):
        r = i * T if isinstance(i, int) else pl.multiple_of(i * T, T)
        return pltpu.make_async_copy(o_v.at[pl.ds(r, T), :], o_hbm.at[0, pl.ds(r, T), :], sem_o.at[i])

    def cp_cols(src, dst, lo, hi, sem):
        return pltpu.make_async_copy(src.at[:, lo:hi], dst.at[:, lo:hi], sem_w.at[sem])

    cps = {}
    for i in range(NT):
        cps['x%d' % i] = pltpu.make_async_copy(
            x_hbm.at[0, pl.ds(i * T, T), :], x_v.at[pl.ds(i * T, T), :], sem_x.at[i])
    cps['wk'] = cp_cols(wa_hbm, wa_v, 512, 768, 0)
    cps['wk2'] = cp_cols(wa_hbm, wa_v, 768, 1024, 9)
    cps['wq'] = cp_cols(wa_hbm, wa_v, 0, 512, 1)
    cps['wv'] = cp_cols(wa_hbm, wa_v, 1024, 1536, 6)
    for m in range(3):
        cps['wb%d' % m] = cp_cols(wb_hbm, wb_v, m * 512, (m + 1) * 512, 2 + m)
    cps['wob'] = pltpu.make_async_copy(wob_hbm, wob_v, sem_w.at[5])
    cps['woa'] = pltpu.make_async_copy(woa_hbm, woa_v, sem_w.at[7])
    cps['gw'] = pltpu.make_async_copy(gw_hbm, gw_ref, sem_w.at[8])

    cpz = pltpu.make_async_copy(zero_hbm, zero_s, sem_w.at[10])
    cpz.start()
    for n in SCHED[0][0] + ['wk2']:
        cps[n].start()
    cpz.wait()
    dz8 = 8 * zero_s[0]
    for ci, cv in enumerate([QSCALE, 0.0, 1.0, LOG2E, -3.0e38]):
        cb[8 * ci:8 * ci + 8, :] = jnp.full((8, 128), cv, F32)

    def token(tok):
        cb[pl.ds(pl.multiple_of(40 + dz8, 8), 8), :] = tok

    def deadline(ref):
        val = ref[pl.ds(pl.multiple_of(dz8, 8), 8), 0:128]
        if val.dtype != U32:
            val = pltpu.bitcast(val, U32)
        xu[pl.ds(pl.multiple_of(S // 2 + dz8, 8), 8), 0:128] = val

    def put_padded(tref, c, t, h0=0):
        for h in range(t.shape[0] // 16):
            tref[c, ST * (h0 + h):ST * (h0 + h) + 16, :] = t[16 * h:16 * h + 16, :]

    def gather_perm(tref, c, lo=0, hi=16):
        return jnp.concatenate([tref[c, pl.ds(DD[d], 32, stride=ST), :] for d in range(lo, hi)], axis=0)

    def prep_mat(uref, src_ref, off, m):
        for c in range(2):
            put_padded(uref, c, _pk(src_ref[c * 256:(c + 1) * 256, off:off + 512]).T)
        for c in range(2):
            wcat[m][c * 128:(c + 1) * 128, :] = gather_perm(uref, c).T

    def p1a(i, part=None):
        r0 = i * T
        rows = slice(i * TH, (i + 1) * TH)
        if part != 1:
            xt = x_v[r0:r0 + T, :]
            xu[rows, :] = _pk(xt)
            gw = gw_ref[...].astype(F32).reshape(1, D)
            gl = jnp.sum(xt.astype(F32) * gw, axis=-1, keepdims=True)
            gate_ref[r0:r0 + T, :] = jnp.broadcast_to(jax.nn.sigmoid(gl), (T, 128))
        cols = slice(0, D) if part is None else slice(part * 256, (part + 1) * 256)
        nc = D if part is None else 256
        pk = _phi(jnp.dot(_up(xu[rows, :]), _up(wku[:, cols]), preferred_element_type=F32))
        zs = pk.reshape(T // 8, 8, nc).sum(axis=0)
        pk_ref[rows, cols] = _pk(pk.astype(BF16))
        if i == 0:
            z_ref[:, cols] = zs
        else:
            z_ref[:, cols] += zs

    def p1b(i):
        rows = slice(i * TH, (i + 1) * TH)
        gg = lax.dot_general(_up(pk_ref[rows, :]), _up(xu[rows, :]),
                             (((0,), (0,)), ((), ())), preferred_element_type=F32)
        if i == 0:
            g_ref[...] = gg
        else:
            g_ref[...] += gg
        return [gg[r - 8:r, _cs(c)] for c in range(4) for r in range(128, 513, 128)]

    def mid_pieces():
        row = lax.broadcasted_iota(jnp.int32, (128, 128), 0)
        col = lax.broadcasted_iota(jnp.int32, (128, 128), 1)
        same_head = (row // DH) == (col // DH)

        def f1():
            toks = []
            for c in range(4):
                kv = jnp.dot(g_ref[_cs(c), :].astype(BF16), wa_v[:, _cs(8 + c)], preferred_element_type=F32)
                kv_ref[c] = _pk(jnp.where(same_head, kv, 0.0).astype(BF16))
                toks += [kv[56:64, :], kv[120:128, :]]
            return toks

        def f2():
            toks = []
            for c in range(4):
                mm = jnp.dot(_up(kv_ref[c]), woa_v[_cs(c), :], preferred_element_type=F32)
                for c2 in range(4):
                    put_padded(tmp_ref, c2, mm[:, _cs(c2)], h0=8 * c)
                toks += [mm[56:64, 0:128], mm[120:128, 0:128]]
            for c in range(4):
                w2a[:, _cs(c)] = _pk(gather_perm(tmp_ref, c).astype(BF16))
            return toks
        return [(300, f1), (300, f2)]

    def s1_pieces(h0, p, lo, hi):
        n_r = hi - lo

        def piece(n):
            def f():
                m, c = n // 4, n % 4
                res = jnp.dot(_up(xu[pl.ds(h0 + lo // 2, n_r // 2), :]), _up(wcat[m][:, _cs(c)]),
                              preferred_element_type=F32)
                if m < 2:
                    qq[p][lo:hi, _cs(n)] = res
                else:
                    (kb if m == 2 else vb)[p][c, HALO + lo:HALO + hi, :] = res
                return [res[r - 8:r, :] for r in range(TOKROWS, n_r + 1, TOKROWS)]
            return (n_r, f)
        return [piece(n) for n in range(16)]

    def s3_pieces(r0, p, lo=0, hi=T):
        n_r = hi - lo

        def piece(n):
            def f():
                res1 = jnp.dot(_up(lhs[p][lo // 2:hi // 2, 0:512]), _up(w2a[:, _cs(n)]),
                               preferred_element_type=F32)
                res = res1 + jnp.dot(_up(lhs[p][lo // 2:hi // 2, 512:1024]), _up(w2b[:, _cs(n)]),
                                     preferred_element_type=F32)
                o_v[pl.ds(r0 + lo, n_r), _cs(n)] = res.astype(BF16)
                return ([res1[r - 8:r, :] for r in range(TOKROWS, n_r + 1, TOKROWS)]
                        + [res[r - 8:r, :] for r in range(TOKROWS, n_r + 1, TOKROWS)])
            return (2 * n_r, f)
        return [piece(n) for n in range(4)]

    def halo(p):
        for c in range(4):
            kb[p][c, 0:HALO, :] = kb[1 - p][c, T:T + HALO, :]
            vb[p][c, 0:HALO, :] = vb[1 - p][c, T:T + HALO, :]

    def s2_parts(r0, p, first):
        pend = {}

        def put(rs, c0, vals):
            if rs % 16 == 0:
                pend[c0] = vals
            else:
                prev = pend.pop(c0)
                r2 = (rs - 8) // 2
                for c in range(4):
                    lhs[p][r2:r2 + 8, _cs(c0 + c)] = _pk(
                        jnp.concatenate([prev[c], vals[c]], axis=0).astype(BF16))

        def group(rs):
            st = {}

            def part_a():
                g = gate_ref[pl.ds(r0 + rs, R), :]
                st['g'] = g
                c0, c1, cl = cb[8:16, :], cb[16:24, :], cb[24:32, :]
                pq = []
                for c in range(4):
                    tq = qq[p][rs:rs + R, _cs(c)]
                    pq.append(jnp.where(tq > c0, tq + c1, jnp.exp2(tq * cl)) + 1e-6)
                t = pq[0] * z_ref[:, _cs(0)]
                for c in range(1, 4):
                    t = t + pq[c] * z_ref[:, _cs(c)]
                sa = g * _recip(_group_sum(t) + 1e-6)
                put(rs, 0, [pq[c] * sa for c in range(4)])

            def part_qk():
                sc = cb[0:8, :]
                q = [qq[p][rs:rs + R, _cs(4 + c)] * sc for c in range(4)]
                ls = []
                for w in range(W):
                    k0_ = HALO + rs - DIL * w
                    pp = q[0] * kb[p][0, k0_:k0_ + R, :]
                    for c in range(1, 4):
                        pp = pp + q[c] * kb[p][c, k0_:k0_ + R, :]
                    pp = _group_sum(pp)
                    if first and rs < DIL * w:
                        rowi = rs + lax.broadcasted_iota(jnp.int32, (R, 128), 0)
                        pp = jnp.where(rowi >= DIL * w, pp, -1e9)
                    ls.append(pp)
                m = ls[0]
                for w in range(1, W):
                    m = jnp.maximum(m, ls[w])
                st['ls'], st['m'] = ls, m

            def part_av():
                m = jnp.maximum(st['m'], cb[32:40, :])
                es = [jnp.exp2(l - m) for l in st['ls']]
                ssum = es[0]
                for w in range(1, W):
                    ssum = ssum + es[w]
                sb = (1.0 - st['g']) * _recip(ssum)
                outs = []
                for c in range(4):
                    o = es[0] * vb[p][c, HALO + rs:HALO + rs + R, :]
                    for w in range(1, W):
                        v0_ = HALO + rs - DIL * w
                        o = o + es[w] * vb[p][c, v0_:v0_ + R, :]
                    outs.append(o * sb)
                put(rs, 4, outs)

            return (part_a, part_qk, part_av)

        seq = []
        for rs in range(0, T, 2 * R):
            pair = (group(rs), group(rs + R))
            seq += [pair[j][kind] for kind, j in PATTERN]
        return seq

    def emit(mx, vp, tailcyc, ngate, gate_cyc):
        span = max(sum(c for c, _ in mx) - tailcyc, 1)
        nv = len(vp)
        vp[0]()
        done, cyc = 1, 0
        for c, f in mx:
            toks = f()
            for ti, tok in enumerate(toks):
                now = cyc + c * (ti + 1) / len(toks)
                upto = min(nv, 1 + int((nv - 1) * now / span + 0.5))
                if now < gate_cyc:
                    upto = min(upto, ngate)
                if upto > done:
                    token(tok)
                    for g_ in vp[done:upto]:
                        g_()
                    done = upto
            cyc += c
        for g_ in vp[done:]:
            g_()

    def step(h_cur, h_next, r_cur, r_prev, p, first=False, tailcyc=TAILCYC):
        mx = s1_pieces(h_cur, p, HT, T)
        gate_cyc = sum(c for c, _ in mx)
        if first:
            mx += [(600, lambda: p1b(NT - 2)), (600, lambda: p1b(NT - 1))]
        if r_prev is not None:
            mx += s3_pieces(r_prev, 1 - p)
        if h_next is not None:
            nxt = s1_pieces(h_next, 1 - p, 0, HT)
            c0, f0 = nxt[0]

            def f0h():
                halo(1 - p)
                return f0()
            nxt = [(c0, f0h)] + nxt[1:]
            if first:
                mid = mid_pieces()
                nxt = nxt[:3] + [mid[0]] + nxt[3:8] + [mid[1]] + nxt[8:]
            mx += nxt
        emit(mx, s2_parts(r_cur, p, first), tailcyc, 3 * (HT // R), gate_cyc)

    def do_work(wk):
        if wk == 'rk0':
            wku[:, 0:256] = _pk(wa_v[:, 512:768])
        elif wk == 'rk1':
            wku[:, 256:512] = _pk(wa_v[:, 768:1024])
        elif wk == 'A0':
            p1a(0, 0)
        elif wk == 'B0':
            p1a(0, 1)
        elif wk[0] == 'a':
            p1a(int(wk[1:]))
        elif wk[0] == 'b':
            p1b(int(wk[1:]))
        elif wk == 'g':
            deadline(gate_ref)
        elif wk[0] == 'd':
            deadline(wcat[int(wk[1:])])
        elif wk == 'pq':
            prep_mat(ut0, wa_v, 0, 0)
        else:
            m = int(wk[1:])
            prep_mat(ut1 if m % 2 == 0 else ut0, wb_v, m * 512, m + 1)

    for waits, issues, work in SCHED:
        for n in waits:
            cps[n].wait()
        for n in issues:
            cps[n].start()
        for wk in work:
            do_work(wk)

    z = jnp.broadcast_to(jnp.sum(z_ref[...], axis=0, keepdims=True), (8, D))
    zc = _lane_perm([z[:, _cs(c)] for c in range(4)])
    for c in range(4):
        z_ref[:, _cs(c)] = zc[c]
        kb[0][c, 0:HALO, :] = jnp.zeros((HALO, 128), F32)
        vb[0][c, 0:HALO, :] = jnp.zeros((HALO, 128), F32)

    po_tasks = []
    for c in range(4):
        for q4 in range(4):
            po_tasks.append(lambda c=c, q4=q4: put_padded(
                tmp2_ref, c, wob_v[q4 * 128:(q4 + 1) * 128, _cs(c)].astype(F32), h0=8 * q4))
        for q4 in range(4):
            def t2(c=c, q4=q4):
                w2b[q4 * 64:(q4 + 1) * 64, _cs(c)] = _pk(gather_perm(tmp2_ref, c, 4 * q4, 4 * q4 + 4).astype(BF16))
            po_tasks.append(t2)
    for pi, (_, f) in enumerate(s1_pieces(0, 0, 0, HT)):
        if pi == 4:
            deadline(wcat[3])
        toks = f()
        for ti, tok in enumerate(toks[len(toks) // 2 - 1::len(toks) // 2]):
            tmp2_ref[0, pl.ds(pl.multiple_of(32 * ST + dz8, 8), 8), :] = tok
            po_tasks[2 * pi + ti]()

    step(0, TH, 0, None, 0, first=True, tailcyc=768)

    def pair_body(j, carry):
        i1 = 2 * j + 1
        r1 = pl.multiple_of(i1 * T, T)
        h2 = pl.multiple_of((i1 + 1) * TH, TH)
        step(pl.multiple_of(i1 * TH, TH), h2, r1, pl.multiple_of(r1 - T, T), 1)
        cp_o(i1 - 1).start()
        step(h2, pl.multiple_of((i1 + 2) * TH, TH), pl.multiple_of(r1 + T, T), r1, 0)
        cp_o(i1).start()
        return carry

    lax.fori_loop(0, (NT - 2) // 2, pair_body, 0)

    rl = (NT - 1) * T
    step((NT - 1) * TH, None, rl, rl - T, 1, tailcyc=0)
    cp_o(NT - 2).start()

    def cp_last(lo, cols, sem):
        return pltpu.make_async_copy(o_v.at[pl.ds(rl + lo, HT), cols], o_hbm.at[0, pl.ds(rl + lo, HT), cols],
                                     sem_o.at[sem])

    last = [cp_last(0, slice(0, D), NT - 1), cp_last(HT, slice(0, 384), NT), cp_last(HT, slice(384, D), NT + 1)]
    for _, f in s3_pieces(rl, 1, 0, HT):
        f()
    last[0].start()
    for n, (_, f) in enumerate(s3_pieces(rl, 1, HT, T)):
        f()
        if n >= 2:
            last[n - 1].start()
    for i in range(NT - 1):
        cp_o(i).wait()
    for c_ in last:
        c_.wait()


@jax.jit
def pallas_gated_mix__linear_attn_block__sliding_local_dilated__prompt_kernel(A_x, A_wqkv, A_wo, B_x, B_wqkv, B_wo, gate_w):
    anyspec = pl.BlockSpec(memory_space=pl.ANY)
    two = lambda shape, dt: [pltpu.VMEM(shape, dt)] * 2
    return pl.pallas_call(
        _kernel,
        grid=(1,),
        in_specs=[anyspec] * 7,
        out_specs=anyspec,
        out_shape=jax.ShapeDtypeStruct((1, S, D), BF16),
        scratch_shapes=[
            pltpu.SMEM((8,), jnp.int32),
            pltpu.VMEM((D,), BF16),
            pltpu.VMEM((S, D), BF16),
            pltpu.VMEM((D, 3 * D), BF16),
            pltpu.VMEM((D, D), BF16),
            pltpu.VMEM((D, 3 * D), BF16),
            pltpu.VMEM((D, D), BF16),
            pltpu.VMEM((S, D), BF16),
            pltpu.VMEM((S // 2 + 8, D), U32),
            pltpu.VMEM((D // 2, D), U32),
            *two((D // 2, D), U32), *two((D // 2, D), U32),
            *two((D // 2, D), U32),
            pltpu.VMEM((4, 64, 128), U32),
            pltpu.VMEM((D, D), F32),
            pltpu.VMEM((8, D), F32),
            pltpu.VMEM((4, 32 * ST, 128), F32),
            pltpu.VMEM((4, 32 * ST + 8, 128), F32),
            *two((2, 32 * ST, 128), U32),
            pltpu.VMEM((S, 128), F32),
            pltpu.VMEM((S // 2, D), U32),
            *two((T, 2 * D), F32),
            *two((4, HALO + T, 128), F32),
            *two((4, HALO + T, 128), F32),
            *two((T // 2, 2 * D), U32),
            pltpu.VMEM((48, 128), F32),
            pltpu.SemaphoreType.DMA((NT,)),
            pltpu.SemaphoreType.DMA((11,)),
            pltpu.SemaphoreType.DMA((NT + 2,)),
        ],
        compiler_params=pltpu.CompilerParams(vmem_limit_bytes=100 * 1024 * 1024),
    )(A_x, A_wqkv, A_wo, B_wqkv, B_wo, gate_w, jnp.zeros((8,), jnp.int32))
```

```python
import jax
import jax.numpy as jnp
from jax import lax
import jax.experimental.pallas as pl
import jax.experimental.pallas.tpu as pltpu

S, D, DH, W, DIL = 2048, 512, 16, 8, 2
T = 256
TH = T // 2
HT = T // 2
NT = S // T
R = 8
HALO = 16
ST = 20
SWAPS = [(1, 4), (1, 0), (1, 5), (1, 1), (0, 3), (0, 6), (0, 2)]
DD = [((d >> 1) & 1) * 8 + ((d >> 2) & 1) * 4 + ((d >> 3) & 1) * 2 + (d & 1) for d in range(16)]
F32, BF16, U32 = jnp.float32, jnp.bfloat16, jnp.uint32
LOG2E = 1.4426950408889634
QSCALE = (DH ** -0.5) * LOG2E
M1, M2 = 3, 7
TOKROWS = 32
TAILCYC = 512
PATTERN = ((1, 0), (1, 1), (0, 0), (0, 1), (2, 0), (2, 1))
SCHED = [
    (['gw', 'x0', 'wk'], ['x1', 'x2', 'x3'], ['rk0', 'A0']),
    (['wk2'], ['x4', 'x5'], ['rk1', 'B0', 'b0']),
    (['x1', 'x2', 'x3'], ['wq', 'wb0', 'x6', 'x7', 'wb1', 'wb2'], ['a1', 'a2', 'b1', 'g', 'a3', 'g', 'b2']),
    (['x4', 'x5', 'wq', 'wb0'], ['wob', 'wv', 'woa'], ['pq', 'p0', 'a4', 'b3', 'd0', 'a5', 'g', 'd1', 'b4']),
    (['x6', 'x7', 'wb1', 'wb2', 'wob', 'wv', 'woa'], [], ['p1', 'p2', 'a6', 'b5', 'd2', 'a7', 'g']),
]


def _phi(t):
    return jnp.where(t > 0, t + 1.0, jnp.exp(t)) + 1e-6


def _recip(x):
    r = pl.reciprocal(x, approx=True)
    return r * (2.0 - x * r)


def _lane_perm(chunks):
    lane = lax.broadcasted_iota(jnp.int32, chunks[0].shape, 1)
    chunks = list(chunks)
    for cbit, j in SWAPS:
        bit = ((lane >> j) & 1) == 1
        out = list(chunks)
        for c in range(4):
            if (c >> cbit) & 1 == 0:
                a = chunks[c]
                b = chunks[c | (1 << cbit)]
                out[c] = jnp.where(bit, pltpu.roll(b, 1 << j, 1), a)
                out[c | (1 << cbit)] = jnp.where(bit, b, pltpu.roll(a, 128 - (1 << j), 1))
        chunks = out
    return chunks


def _group_sum(p):
    p = p + pltpu.roll(p, 32, 1)
    return p + pltpu.roll(p, 64, 1)


def _cs(c):
    return slice(c * 128, (c + 1) * 128)


def _pk(x):
    return pltpu.bitcast(x, U32)


def _up(u):
    return pltpu.bitcast(u, BF16)


def _kernel(x_hbm, wa_hbm, woa_hbm, wb_hbm, wob_hbm, gw_hbm, zero_hbm, o_hbm,
            zero_s, gw_ref, x_v, wa_v, woa_v, wb_v, wob_v, o_v,
            xu, wku, wc0, wc1, wc2, wc3, w2a, w2b, kv_ref, g_ref, z_ref, tmp_ref, tmp2_ref, ut0, ut1,
            gate_ref, pk_ref, qq0, qq1, k0, k1, v0, v1, lhs0, lhs1, cb, sem_x, sem_w, sem_o):
    qq, kb, vb, lhs = (qq0, qq1), (k0, k1), (v0, v1), (lhs0, lhs1)
    wcat = (wc0, wc1, wc2, wc3)

    def cp_o(i):
        r = i * T if isinstance(i, int) else pl.multiple_of(i * T, T)
        return pltpu.make_async_copy(o_v.at[pl.ds(r, T), :], o_hbm.at[0, pl.ds(r, T), :], sem_o.at[i])

    def cp_cols(src, dst, lo, hi, sem):
        return pltpu.make_async_copy(src.at[:, lo:hi], dst.at[:, lo:hi], sem_w.at[sem])

    cps = {}
    for i in range(NT):
        cps['x%d' % i] = pltpu.make_async_copy(
            x_hbm.at[0, pl.ds(i * T, T), :], x_v.at[pl.ds(i * T, T), :], sem_x.at[i])
    cps['wk'] = cp_cols(wa_hbm, wa_v, 512, 768, 0)
    cps['wk2'] = cp_cols(wa_hbm, wa_v, 768, 1024, 9)
    cps['wq'] = cp_cols(wa_hbm, wa_v, 0, 512, 1)
    cps['wv'] = cp_cols(wa_hbm, wa_v, 1024, 1536, 6)
    for m in range(3):
        cps['wb%d' % m] = cp_cols(wb_hbm, wb_v, m * 512, (m + 1) * 512, 2 + m)
    cps['wob'] = pltpu.make_async_copy(wob_hbm, wob_v, sem_w.at[5])
    cps['woa'] = pltpu.make_async_copy(woa_hbm, woa_v, sem_w.at[7])
    cps['gw'] = pltpu.make_async_copy(gw_hbm, gw_ref, sem_w.at[8])

    cpz = pltpu.make_async_copy(zero_hbm, zero_s, sem_w.at[10])
    cpz.start()
    for n in SCHED[0][0] + ['wk2']:
        cps[n].start()
    cpz.wait()
    dz8 = 8 * zero_s[0]
    for ci, cv in enumerate([QSCALE, 0.0, 1.0, LOG2E, -3.0e38]):
        cb[8 * ci:8 * ci + 8, :] = jnp.full((8, 128), cv, F32)

    def token(tok):
        cb[pl.ds(pl.multiple_of(40 + dz8, 8), 8), :] = tok

    def deadline(ref):
        val = ref[pl.ds(pl.multiple_of(dz8, 8), 8), 0:128]
        if val.dtype != U32:
            val = pltpu.bitcast(val, U32)
        xu[pl.ds(pl.multiple_of(S // 2 + dz8, 8), 8), 0:128] = val

    def put_padded(tref, c, t, h0=0):
        for h in range(t.shape[0] // 16):
            tref[c, ST * (h0 + h):ST * (h0 + h) + 16, :] = t[16 * h:16 * h + 16, :]

    def gather_perm(tref, c, lo=0, hi=16):
        return jnp.concatenate([tref[c, pl.ds(DD[d], 32, stride=ST), :] for d in range(lo, hi)], axis=0)

    def prep_mat(uref, src_ref, off, m):
        for c in range(2):
            put_padded(uref, c, _pk(src_ref[c * 256:(c + 1) * 256, off:off + 512]).T)
        for c in range(2):
            wcat[m][c * 128:(c + 1) * 128, :] = gather_perm(uref, c).T

    def p1a(i, part=None):
        r0 = i * T
        rows = slice(i * TH, (i + 1) * TH)
        if part != 1:
            xt = x_v[r0:r0 + T, :]
            xu[rows, :] = _pk(xt)
            gw = gw_ref[...].astype(F32).reshape(1, D)
            gl = jnp.sum(xt.astype(F32) * gw, axis=-1, keepdims=True)
            gate_ref[r0:r0 + T, :] = jnp.broadcast_to(jax.nn.sigmoid(gl), (T, 128))
        cols = slice(0, D) if part is None else slice(part * 256, (part + 1) * 256)
        nc = D if part is None else 256
        pk = _phi(jnp.dot(_up(xu[rows, :]), _up(wku[:, cols]), preferred_element_type=F32))
        zs = pk.reshape(T // 8, 8, nc).sum(axis=0)
        pk_ref[rows, cols] = _pk(pk.astype(BF16))
        if i == 0:
            z_ref[:, cols] = zs
        else:
            z_ref[:, cols] += zs

    def p1b(i):
        rows = slice(i * TH, (i + 1) * TH)
        gg = lax.dot_general(_up(pk_ref[rows, :]), _up(xu[rows, :]),
                             (((0,), (0,)), ((), ())), preferred_element_type=F32)
        if i == 0:
            g_ref[...] = gg
        else:
            g_ref[...] += gg
        return [gg[r - 8:r, _cs(c)] for c in range(4) for r in range(128, 513, 128)]

    def mid_pieces():
        row = lax.broadcasted_iota(jnp.int32, (128, 128), 0)
        col = lax.broadcasted_iota(jnp.int32, (128, 128), 1)
        same_head = (row // DH) == (col // DH)

        def f1():
            toks = []
            for c in range(4):
                kv = jnp.dot(g_ref[_cs(c), :].astype(BF16), wa_v[:, _cs(8 + c)], preferred_element_type=F32)
                kv_ref[c] = _pk(jnp.where(same_head, kv, 0.0).astype(BF16))
                toks += [kv[56:64, :], kv[120:128, :]]
            return toks

        def f2():
            toks = []
            for c in range(4):
                mm = jnp.dot(_up(kv_ref[c]), woa_v[_cs(c), :], preferred_element_type=F32)
                for c2 in range(4):
                    put_padded(tmp_ref, c2, mm[:, _cs(c2)], h0=8 * c)
                toks += [mm[56:64, 0:128], mm[120:128, 0:128]]
            return toks
        return [(300, f1), (300, f2)]

    def with_m_perm(piece, j):
        c_, f = piece

        def g():
            toks = f()
            for ti, tok in enumerate(toks[len(toks) // 2 - 1::len(toks) // 2]):
                c, q4 = (2 * j + ti) // 4, (2 * j + ti) % 4
                tmp_ref[0, pl.ds(pl.multiple_of(32 * ST + dz8, 8), 8), :] = tok
                w2a[q4 * 64:(q4 + 1) * 64, _cs(c)] = _pk(gather_perm(tmp_ref, c, 4 * q4, 4 * q4 + 4).astype(BF16))
            return toks
        return (c_, g)

    def s1_pieces(h0, p, lo, hi):
        n_r = hi - lo

        def piece(n):
            def f():
                m, c = n // 4, n % 4
                res = jnp.dot(_up(xu[pl.ds(h0 + lo // 2, n_r // 2), :]), _up(wcat[m][:, _cs(c)]),
                              preferred_element_type=F32)
                if m < 2:
                    qq[p][lo:hi, _cs(n)] = res
                else:
                    (kb if m == 2 else vb)[p][c, HALO + lo:HALO + hi, :] = res
                return [res[r - 8:r, :] for r in range(TOKROWS, n_r + 1, TOKROWS)]
            return (n_r, f)
        return [piece(n) for n in range(16)]

    def s3_pieces(r0, p, lo=0, hi=T):
        n_r = hi - lo

        def piece(n):
            def f():
                res1 = jnp.dot(_up(lhs[p][lo // 2:hi // 2, 0:512]), _up(w2a[:, _cs(n)]),
                               preferred_element_type=F32)
                res = res1 + jnp.dot(_up(lhs[p][lo // 2:hi // 2, 512:1024]), _up(w2b[:, _cs(n)]),
                                     preferred_element_type=F32)
                o_v[pl.ds(r0 + lo, n_r), _cs(n)] = res.astype(BF16)
                return ([res1[r - 8:r, :] for r in range(TOKROWS, n_r + 1, TOKROWS)]
                        + [res[r - 8:r, :] for r in range(TOKROWS, n_r + 1, TOKROWS)])
            return (2 * n_r, f)
        return [piece(n) for n in range(4)]

    def halo(p):
        for c in range(4):
            kb[p][c, 0:HALO, :] = kb[1 - p][c, T:T + HALO, :]
            vb[p][c, 0:HALO, :] = vb[1 - p][c, T:T + HALO, :]

    def s2_parts(r0, p, first):
        pend = {}

        def put(rs, c0, vals):
            if rs % 16 == 0:
                pend[c0] = vals
            else:
                prev = pend.pop(c0)
                r2 = (rs - 8) // 2
                for c in range(4):
                    lhs[p][r2:r2 + 8, _cs(c0 + c)] = _pk(
                        jnp.concatenate([prev[c], vals[c]], axis=0).astype(BF16))

        def group(rs):
            st = {}

            def part_a():
                g = gate_ref[pl.ds(r0 + rs, R), :]
                st['g'] = g
                c0, c1, cl = cb[8:16, :], cb[16:24, :], cb[24:32, :]
                pq = []
                for c in range(4):
                    tq = qq[p][rs:rs + R, _cs(c)]
                    pq.append(jnp.where(tq > c0, tq + c1, jnp.exp2(tq * cl)) + 1e-6)
                t = pq[0] * z_ref[:, _cs(0)]
                for c in range(1, 4):
                    t = t + pq[c] * z_ref[:, _cs(c)]
                sa = g * _recip(_group_sum(t) + 1e-6)
                put(rs, 0, [pq[c] * sa for c in range(4)])

            def part_qk():
                sc = cb[0:8, :]
                q = [qq[p][rs:rs + R, _cs(4 + c)] * sc for c in range(4)]
                ls = []
                for w in range(W):
                    k0_ = HALO + rs - DIL * w
                    pp = q[0] * kb[p][0, k0_:k0_ + R, :]
                    for c in range(1, 4):
                        pp = pp + q[c] * kb[p][c, k0_:k0_ + R, :]
                    pp = _group_sum(pp)
                    if first and rs < DIL * w:
                        rowi = rs + lax.broadcasted_iota(jnp.int32, (R, 128), 0)
                        pp = jnp.where(rowi >= DIL * w, pp, -1e9)
                    ls.append(pp)
                m = ls[0]
                for w in range(1, W):
                    m = jnp.maximum(m, ls[w])
                st['ls'], st['m'] = ls, m

            def part_av():
                m = jnp.maximum(st['m'], cb[32:40, :])
                es = [jnp.exp2(l - m) for l in st['ls']]
                ssum = es[0]
                for w in range(1, W):
                    ssum = ssum + es[w]
                sb = (1.0 - st['g']) * _recip(ssum)
                outs = []
                for c in range(4):
                    o = es[0] * vb[p][c, HALO + rs:HALO + rs + R, :]
                    for w in range(1, W):
                        v0_ = HALO + rs - DIL * w
                        o = o + es[w] * vb[p][c, v0_:v0_ + R, :]
                    outs.append(o * sb)
                put(rs, 4, outs)

            return (part_a, part_qk, part_av)

        seq = []
        for rs in range(0, T, 2 * R):
            pair = (group(rs), group(rs + R))
            seq += [pair[j][kind] for kind, j in PATTERN]
        return seq

    def emit(mx, vp, tailcyc, ngate, gate_cyc):
        span = max(sum(c for c, _ in mx) - tailcyc, 1)
        nv = len(vp)
        vp[0]()
        done, cyc = 1, 0
        for c, f in mx:
            toks = f()
            for ti, tok in enumerate(toks):
                now = cyc + c * (ti + 1) / len(toks)
                upto = min(nv, 1 + int((nv - 1) * now / span + 0.5))
                if now < gate_cyc:
                    upto = min(upto, ngate)
                if upto > done:
                    token(tok)
                    for g_ in vp[done:upto]:
                        g_()
                    done = upto
            cyc += c
        for g_ in vp[done:]:
            g_()

    def step(h_cur, h_next, r_cur, r_prev, p, first=False, tailcyc=TAILCYC):
        mx = s1_pieces(h_cur, p, HT, T)
        gate_cyc = sum(c for c, _ in mx)
        if first:
            mx += [(600, lambda: p1b(NT - 2)), (600, lambda: p1b(NT - 1))]
        if r_prev is not None:
            mx += s3_pieces(r_prev, 1 - p)
        if h_next is not None:
            nxt = s1_pieces(h_next, 1 - p, 0, HT)
            c0, f0 = nxt[0]

            def f0h():
                halo(1 - p)
                return f0()
            nxt = [(c0, f0h)] + nxt[1:]
            if first:
                mid = mid_pieces()
                nxt = (nxt[:M1] + [mid[0]] + nxt[M1:M2] + [mid[1]]
                       + [with_m_perm(pc, j) for j, pc in enumerate(nxt[M2:M2 + 8])] + nxt[M2 + 8:])
            mx += nxt
        emit(mx, s2_parts(r_cur, p, first), tailcyc, 3 * (HT // R), gate_cyc)

    def do_work(wk):
        if wk == 'rk0':
            wku[:, 0:256] = _pk(wa_v[:, 512:768])
        elif wk == 'rk1':
            wku[:, 256:512] = _pk(wa_v[:, 768:1024])
        elif wk == 'A0':
            p1a(0, 0)
        elif wk == 'B0':
            p1a(0, 1)
        elif wk[0] == 'a':
            p1a(int(wk[1:]))
        elif wk[0] == 'b':
            p1b(int(wk[1:]))
        elif wk == 'g':
            deadline(gate_ref)
        elif wk[0] == 'd':
            deadline(wcat[int(wk[1:])])
        elif wk == 'pq':
            prep_mat(ut0, wa_v, 0, 0)
        else:
            m = int(wk[1:])
            prep_mat(ut1 if m % 2 == 0 else ut0, wb_v, m * 512, m + 1)

    for waits, issues, work in SCHED:
        for n in waits:
            cps[n].wait()
        for n in issues:
            cps[n].start()
        for wk in work:
            do_work(wk)

    z = jnp.broadcast_to(jnp.sum(z_ref[...], axis=0, keepdims=True), (8, D))
    zc = _lane_perm([z[:, _cs(c)] for c in range(4)])
    for c in range(4):
        z_ref[:, _cs(c)] = zc[c]
        kb[0][c, 0:HALO, :] = jnp.zeros((HALO, 128), F32)
        vb[0][c, 0:HALO, :] = jnp.zeros((HALO, 128), F32)

    po_tasks = []
    for c in range(4):
        for q4 in range(4):
            po_tasks.append(lambda c=c, q4=q4: put_padded(
                tmp2_ref, c, wob_v[q4 * 128:(q4 + 1) * 128, _cs(c)].astype(F32), h0=8 * q4))
        for q4 in range(4):
            def t2(c=c, q4=q4):
                w2b[q4 * 64:(q4 + 1) * 64, _cs(c)] = _pk(gather_perm(tmp2_ref, c, 4 * q4, 4 * q4 + 4).astype(BF16))
            po_tasks.append(t2)
    for pi, (_, f) in enumerate(s1_pieces(0, 0, 0, HT)):
        if pi == 4:
            deadline(wcat[3])
        toks = f()
        for ti, tok in enumerate(toks[len(toks) // 2 - 1::len(toks) // 2]):
            tmp2_ref[0, pl.ds(pl.multiple_of(32 * ST + dz8, 8), 8), :] = tok
            po_tasks[2 * pi + ti]()

    step(0, TH, 0, None, 0, first=True, tailcyc=768)

    def pair_body(j, carry):
        i1 = 2 * j + 1
        r1 = pl.multiple_of(i1 * T, T)
        h2 = pl.multiple_of((i1 + 1) * TH, TH)
        step(pl.multiple_of(i1 * TH, TH), h2, r1, pl.multiple_of(r1 - T, T), 1)
        cp_o(i1 - 1).start()
        step(h2, pl.multiple_of((i1 + 2) * TH, TH), pl.multiple_of(r1 + T, T), r1, 0)
        cp_o(i1).start()
        return carry

    lax.fori_loop(0, (NT - 2) // 2, pair_body, 0)

    rl = (NT - 1) * T
    step((NT - 1) * TH, None, rl, rl - T, 1, tailcyc=0)
    cp_o(NT - 2).start()

    def cp_last(lo, cols, sem):
        return pltpu.make_async_copy(o_v.at[pl.ds(rl + lo, HT), cols], o_hbm.at[0, pl.ds(rl + lo, HT), cols],
                                     sem_o.at[sem])

    last = [cp_last(0, slice(0, D), NT - 1), cp_last(HT, slice(0, 384), NT), cp_last(HT, slice(384, D), NT + 1)]
    for _, f in s3_pieces(rl, 1, 0, HT):
        f()
    last[0].start()
    for n, (_, f) in enumerate(s3_pieces(rl, 1, HT, T)):
        f()
        if n >= 2:
            last[n - 1].start()
    for i in range(NT - 1):
        cp_o(i).wait()
    for c_ in last:
        c_.wait()


@jax.jit
def pallas_gated_mix__linear_attn_block__sliding_local_dilated__prompt_kernel(A_x, A_wqkv, A_wo, B_x, B_wqkv, B_wo, gate_w):
    anyspec = pl.BlockSpec(memory_space=pl.ANY)
    two = lambda shape, dt: [pltpu.VMEM(shape, dt)] * 2
    return pl.pallas_call(
        _kernel,
        grid=(1,),
        in_specs=[anyspec] * 7,
        out_specs=anyspec,
        out_shape=jax.ShapeDtypeStruct((1, S, D), BF16),
        scratch_shapes=[
            pltpu.SMEM((8,), jnp.int32),
            pltpu.VMEM((D,), BF16),
            pltpu.VMEM((S, D), BF16),
            pltpu.VMEM((D, 3 * D), BF16),
            pltpu.VMEM((D, D), BF16),
            pltpu.VMEM((D, 3 * D), BF16),
            pltpu.VMEM((D, D), BF16),
            pltpu.VMEM((S, D), BF16),
            pltpu.VMEM((S // 2 + 8, D), U32),
            pltpu.VMEM((D // 2, D), U32),
            *two((D // 2, D), U32), *two((D // 2, D), U32),
            *two((D // 2, D), U32),
            pltpu.VMEM((4, 64, 128), U32),
            pltpu.VMEM((D, D), F32),
            pltpu.VMEM((8, D), F32),
            pltpu.VMEM((4, 32 * ST + 8, 128), F32),
            pltpu.VMEM((4, 32 * ST + 8, 128), F32),
            *two((2, 32 * ST, 128), U32),
            pltpu.VMEM((S, 128), F32),
            pltpu.VMEM((S // 2, D), U32),
            *two((T, 2 * D), F32),
            *two((4, HALO + T, 128), F32),
            *two((4, HALO + T, 128), F32),
            *two((T // 2, 2 * D), U32),
            pltpu.VMEM((48, 128), F32),
            pltpu.SemaphoreType.DMA((NT,)),
            pltpu.SemaphoreType.DMA((11,)),
            pltpu.SemaphoreType.DMA((NT + 2,)),
        ],
        compiler_params=pltpu.CompilerParams(vmem_limit_bytes=100 * 1024 * 1024),
    )(A_x, A_wqkv, A_wo, B_wqkv, B_wo, gate_w, jnp.zeros((8,), jnp.int32))
```

```python
import jax
import jax.numpy as jnp
from jax import lax
import jax.experimental.pallas as pl
import jax.experimental.pallas.tpu as pltpu

S, D, DH, W, DIL = 2048, 512, 16, 8, 2
T = 256
TH = T // 2
HT = T // 2
NT = S // T
R = 8
HALO = 16
ST = 20
SWAPS = [(1, 4), (1, 0), (1, 5), (1, 1), (0, 3), (0, 6), (0, 2)]
DD = [((d >> 1) & 1) * 8 + ((d >> 2) & 1) * 4 + ((d >> 3) & 1) * 2 + (d & 1) for d in range(16)]
F32, BF16, U32 = jnp.float32, jnp.bfloat16, jnp.uint32
LOG2E = 1.4426950408889634
QSCALE = (DH ** -0.5) * LOG2E
M1, M2 = 3, 7
TOKROWS = 32
TAILCYC = 512
PATTERN = ((1, 0), (1, 1), (0, 0), (0, 1), (2, 0), (2, 1))
SCHED = [
    (['gw', 'x0', 'wk'], ['x1', 'x2', 'x3'], ['rk0', 'A0']),
    (['wk2'], ['x4', 'x5'], ['rk1', 'B0', 'b0']),
    (['x1', 'x2', 'x3'], ['wq', 'wb0', 'x6', 'x7', 'wb1', 'wb2'], ['a1', 'a2', 'b1', 'g', 'a3', 'g', 'b2']),
    (['x4', 'x5', 'wq', 'wb0'], ['wob', 'wv', 'woa'], ['pq', 'p0', 'a4', 'b3', 'd0', 'a5', 'g', 'd1', 'b4']),
    (['x6', 'x7', 'wb1', 'wb2', 'wob', 'wv', 'woa'], [], ['p1', 'p2', 'a6', 'b5', 'd2', 'a7', 'g']),
]


def _phi(t):
    return jnp.where(t > 0, t + 1.0, jnp.exp(t)) + 1e-6


def _recip(x):
    r = pl.reciprocal(x, approx=True)
    return r * (2.0 - x * r)


def _lane_perm(chunks):
    lane = lax.broadcasted_iota(jnp.int32, chunks[0].shape, 1)
    chunks = list(chunks)
    for cbit, j in SWAPS:
        bit = ((lane >> j) & 1) == 1
        out = list(chunks)
        for c in range(4):
            if (c >> cbit) & 1 == 0:
                a = chunks[c]
                b = chunks[c | (1 << cbit)]
                out[c] = jnp.where(bit, pltpu.roll(b, 1 << j, 1), a)
                out[c | (1 << cbit)] = jnp.where(bit, b, pltpu.roll(a, 128 - (1 << j), 1))
        chunks = out
    return chunks


def _group_sum(p):
    p = p + pltpu.roll(p, 32, 1)
    return p + pltpu.roll(p, 64, 1)


def _cs(c):
    return slice(c * 128, (c + 1) * 128)


def _pk(x):
    return pltpu.bitcast(x, U32)


def _up(u):
    return pltpu.bitcast(u, BF16)


def _kernel(x_hbm, wa_hbm, woa_hbm, wb_hbm, wob_hbm, gw_hbm, zero_hbm, o_hbm,
            zero_s, gw_ref, x_v, wa_v, woa_v, wb_v, wob_v, o_v,
            xu, wku, wc0, wc1, wc2, wc3, w2a, w2b, kv_ref, g_ref, z_ref, tmp_ref, tmp2_ref, ut0, ut1,
            gate_ref, pk_ref, qq0, qq1, k0, k1, v0, v1, lhs0, lhs1, cb, sem_x, sem_w, sem_o):
    qq, kb, vb, lhs = (qq0, qq1), (k0, k1), (v0, v1), (lhs0, lhs1)
    wcat = (wc0, wc1, wc2, wc3)

    def cp_o(i):
        r = i * T if isinstance(i, int) else pl.multiple_of(i * T, T)
        return pltpu.make_async_copy(o_v.at[pl.ds(r, T), :], o_hbm.at[0, pl.ds(r, T), :], sem_o.at[i])

    def cp_cols(src, dst, lo, hi, sem):
        return pltpu.make_async_copy(src.at[:, lo:hi], dst.at[:, lo:hi], sem_w.at[sem])

    cps = {}
    for i in range(NT):
        cps['x%d' % i] = pltpu.make_async_copy(
            x_hbm.at[0, pl.ds(i * T, T), :], x_v.at[pl.ds(i * T, T), :], sem_x.at[i])
    cps['wk'] = cp_cols(wa_hbm, wa_v, 512, 768, 0)
    cps['wk2'] = cp_cols(wa_hbm, wa_v, 768, 1024, 9)
    cps['wq'] = cp_cols(wa_hbm, wa_v, 0, 512, 1)
    cps['wv'] = cp_cols(wa_hbm, wa_v, 1024, 1536, 6)
    for m in range(3):
        cps['wb%d' % m] = cp_cols(wb_hbm, wb_v, m * 512, (m + 1) * 512, 2 + m)
    cps['wob'] = pltpu.make_async_copy(wob_hbm, wob_v, sem_w.at[5])
    cps['woa'] = pltpu.make_async_copy(woa_hbm, woa_v, sem_w.at[7])
    cps['gw'] = pltpu.make_async_copy(gw_hbm, gw_ref, sem_w.at[8])

    cpz = pltpu.make_async_copy(zero_hbm, zero_s, sem_w.at[10])
    cpz.start()
    for n in SCHED[0][0] + ['wk2']:
        cps[n].start()
    cpz.wait()
    dz8 = 8 * jnp.clip(zero_s[0], 0, 1)
    for ci, cv in enumerate([QSCALE, 0.0, 1.0, LOG2E, -3.0e38]):
        cb[8 * ci:8 * ci + 8, :] = jnp.full((8, 128), cv, F32)

    def token(tok):
        cb[pl.ds(pl.multiple_of(40 + dz8, 8), 8), :] = tok

    def deadline(ref):
        val = ref[pl.ds(pl.multiple_of(dz8, 8), 8), 0:128]
        if val.dtype != U32:
            val = pltpu.bitcast(val, U32)
        xu[pl.ds(pl.multiple_of(S // 2 + dz8, 8), 8), 0:128] = val

    def put_padded(tref, c, t, h0=0):
        for h in range(t.shape[0] // 16):
            tref[c, ST * (h0 + h):ST * (h0 + h) + 16, :] = t[16 * h:16 * h + 16, :]

    def gather_perm(tref, c, lo=0, hi=16):
        return jnp.concatenate([tref[c, pl.ds(DD[d], 32, stride=ST), :] for d in range(lo, hi)], axis=0)

    def prep_mat(uref, src_ref, off, m):
        for c in range(2):
            put_padded(uref, c, _pk(src_ref[c * 256:(c + 1) * 256, off:off + 512]).T)
        for c in range(2):
            wcat[m][c * 128:(c + 1) * 128, :] = gather_perm(uref, c).T

    def p1a(i, part=None):
        r0 = i * T
        rows = slice(i * TH, (i + 1) * TH)
        if part != 1:
            xt = x_v[r0:r0 + T, :]
            xu[rows, :] = _pk(xt)
            gw = gw_ref[...].astype(F32).reshape(1, D)
            gl = jnp.sum(xt.astype(F32) * gw, axis=-1, keepdims=True)
            gate_ref[r0:r0 + T, :] = jnp.broadcast_to(jax.nn.sigmoid(gl), (T, 128))
        cols = slice(0, D) if part is None else slice(part * 256, (part + 1) * 256)
        nc = D if part is None else 256
        pk = _phi(jnp.dot(_up(xu[rows, :]), _up(wku[:, cols]), preferred_element_type=F32))
        zs = pk.reshape(T // 8, 8, nc).sum(axis=0)
        pk_ref[rows, cols] = _pk(pk.astype(BF16))
        if i == 0:
            z_ref[:, cols] = zs
        else:
            z_ref[:, cols] += zs

    def p1b(i):
        rows = slice(i * TH, (i + 1) * TH)
        gg = lax.dot_general(_up(pk_ref[rows, :]), _up(xu[rows, :]),
                             (((0,), (0,)), ((), ())), preferred_element_type=F32)
        if i == 0:
            g_ref[...] = gg
        else:
            g_ref[...] += gg
        return [gg[r - 8:r, _cs(c)] for c in range(4) for r in range(128, 513, 128)]

    def mid_pieces():
        row = lax.broadcasted_iota(jnp.int32, (128, 128), 0)
        col = lax.broadcasted_iota(jnp.int32, (128, 128), 1)
        same_head = (row // DH) == (col // DH)

        def f1():
            toks = []
            for c in range(4):
                kv = jnp.dot(g_ref[_cs(c), :].astype(BF16), wa_v[:, _cs(8 + c)], preferred_element_type=F32)
                kv_ref[c] = _pk(jnp.where(same_head, kv, 0.0).astype(BF16))
                toks += [kv[56:64, :], kv[120:128, :]]
            return toks

        def f2():
            toks = []
            for c in range(4):
                mm = jnp.dot(_up(kv_ref[c]), woa_v[_cs(c), :], preferred_element_type=F32)
                for c2 in range(4):
                    put_padded(tmp_ref, c2, mm[:, _cs(c2)], h0=8 * c)
                toks += [mm[56:64, 0:128], mm[120:128, 0:128]]
            return toks
        return [(300, f1), (300, f2)]

    def with_m_perm(piece, j):
        c_, f = piece

        def g():
            toks = f()
            for ti, tok in enumerate(toks[len(toks) // 2 - 1::len(toks) // 2]):
                c, q4 = (2 * j + ti) // 4, (2 * j + ti) % 4
                tmp_ref[0, pl.ds(pl.multiple_of(32 * ST + dz8, 8), 8), :] = tok
                w2a[q4 * 64:(q4 + 1) * 64, _cs(c)] = _pk(gather_perm(tmp_ref, c, 4 * q4, 4 * q4 + 4).astype(BF16))
            return toks
        return (c_, g)

    def s1_pieces(h0, p, lo, hi):
        n_r = hi - lo

        def piece(n):
            def f():
                m, c = n // 4, n % 4
                res = jnp.dot(_up(xu[pl.ds(h0 + lo // 2, n_r // 2), :]), _up(wcat[m][:, _cs(c)]),
                              preferred_element_type=F32)
                if m < 2:
                    qq[p][lo:hi, _cs(n)] = res
                else:
                    (kb if m == 2 else vb)[p][c, HALO + lo:HALO + hi, :] = res
                return [res[r - 8:r, :] for r in range(TOKROWS, n_r + 1, TOKROWS)]
            return (n_r, f)
        return [piece(n) for n in range(16)]

    def s3_pieces(r0, p, lo=0, hi=T):
        n_r = hi - lo

        def piece(n):
            def f():
                res1 = jnp.dot(_up(lhs[p][lo // 2:hi // 2, 0:512]), _up(w2a[:, _cs(n)]),
                               preferred_element_type=F32)
                res = res1 + jnp.dot(_up(lhs[p][lo // 2:hi // 2, 512:1024]), _up(w2b[:, _cs(n)]),
                                     preferred_element_type=F32)
                o_v[pl.ds(r0 + lo, n_r), _cs(n)] = res.astype(BF16)
                return ([res1[r - 8:r, :] for r in range(TOKROWS, n_r + 1, TOKROWS)]
                        + [res[r - 8:r, :] for r in range(TOKROWS, n_r + 1, TOKROWS)])
            return (2 * n_r, f)
        return [piece(n) for n in range(4)]

    def halo(p):
        for c in range(4):
            kb[p][c, 0:HALO, :] = kb[1 - p][c, T:T + HALO, :]
            vb[p][c, 0:HALO, :] = vb[1 - p][c, T:T + HALO, :]

    def s2_parts(r0, p, first):
        pend = {}

        def put(rs, c0, vals):
            if rs % 16 == 0:
                pend[c0] = vals
            else:
                prev = pend.pop(c0)
                r2 = (rs - 8) // 2
                for c in range(4):
                    lhs[p][r2:r2 + 8, _cs(c0 + c)] = _pk(
                        jnp.concatenate([prev[c], vals[c]], axis=0).astype(BF16))

        def group(rs):
            st = {}

            def part_a():
                g = gate_ref[pl.ds(r0 + rs, R), :]
                st['g'] = g
                c0, c1, cl = cb[8:16, :], cb[16:24, :], cb[24:32, :]
                pq = []
                for c in range(4):
                    tq = qq[p][rs:rs + R, _cs(c)]
                    pq.append(jnp.where(tq > c0, tq + c1, jnp.exp2(tq * cl)) + 1e-6)
                t = pq[0] * z_ref[:, _cs(0)]
                for c in range(1, 4):
                    t = t + pq[c] * z_ref[:, _cs(c)]
                sa = g * _recip(_group_sum(t) + 1e-6)
                put(rs, 0, [pq[c] * sa for c in range(4)])

            def part_qk():
                sc = cb[0:8, :]
                q = [qq[p][rs:rs + R, _cs(4 + c)] * sc for c in range(4)]
                ls = []
                for w in range(W):
                    k0_ = HALO + rs - DIL * w
                    pp = q[0] * kb[p][0, k0_:k0_ + R, :]
                    for c in range(1, 4):
                        pp = pp + q[c] * kb[p][c, k0_:k0_ + R, :]
                    pp = _group_sum(pp)
                    if first and rs < DIL * w:
                        rowi = rs + lax.broadcasted_iota(jnp.int32, (R, 128), 0)
                        pp = jnp.where(rowi >= DIL * w, pp, -1e9)
                    ls.append(pp)
                m = ls[0]
                for w in range(1, W):
                    m = jnp.maximum(m, ls[w])
                st['ls'], st['m'] = ls, m

            def part_av():
                m = jnp.maximum(st['m'], cb[32:40, :])
                es = [jnp.exp2(l - m) for l in st['ls']]
                ssum = es[0]
                for w in range(1, W):
                    ssum = ssum + es[w]
                sb = (1.0 - st['g']) * _recip(ssum)
                outs = []
                for c in range(4):
                    o = es[0] * vb[p][c, HALO + rs:HALO + rs + R, :]
                    for w in range(1, W):
                        v0_ = HALO + rs - DIL * w
                        o = o + es[w] * vb[p][c, v0_:v0_ + R, :]
                    outs.append(o * sb)
                put(rs, 4, outs)

            return (part_a, part_qk, part_av)

        seq = []
        for rs in range(0, T, 2 * R):
            pair = (group(rs), group(rs + R))
            seq += [pair[j][kind] for kind, j in PATTERN]
        return seq

    def emit(mx, vp, tailcyc, ngate, gate_cyc):
        span = max(sum(c for c, _ in mx) - tailcyc, 1)
        nv = len(vp)
        vp[0]()
        done, cyc = 1, 0
        for c, f in mx:
            toks = f()
            for ti, tok in enumerate(toks):
                now = cyc + c * (ti + 1) / len(toks)
                upto = min(nv, 1 + int((nv - 1) * now / span + 0.5))
                if now < gate_cyc:
                    upto = min(upto, ngate)
                if upto > done:
                    token(tok)
                    for g_ in vp[done:upto]:
                        g_()
                    done = upto
            cyc += c
        for g_ in vp[done:]:
            g_()

    def step(h_cur, h_next, r_cur, r_prev, p, first=False, tailcyc=TAILCYC):
        mx = s1_pieces(h_cur, p, HT, T)
        gate_cyc = sum(c for c, _ in mx)
        if first:
            mx += [(600, lambda: p1b(NT - 2)), (600, lambda: p1b(NT - 1))]
        if r_prev is not None:
            mx += s3_pieces(r_prev, 1 - p)
        if h_next is not None:
            nxt = s1_pieces(h_next, 1 - p, 0, HT)
            c0, f0 = nxt[0]

            def f0h():
                halo(1 - p)
                return f0()
            nxt = [(c0, f0h)] + nxt[1:]
            if first:
                mid = mid_pieces()
                nxt = (nxt[:M1] + [mid[0]] + nxt[M1:M2] + [mid[1]]
                       + [with_m_perm(pc, j) for j, pc in enumerate(nxt[M2:M2 + 8])] + nxt[M2 + 8:])
            mx += nxt
        emit(mx, s2_parts(r_cur, p, first), tailcyc, 3 * (HT // R), gate_cyc)

    def do_work(wk):
        if wk == 'rk0':
            wku[:, 0:256] = _pk(wa_v[:, 512:768])
        elif wk == 'rk1':
            wku[:, 256:512] = _pk(wa_v[:, 768:1024])
        elif wk == 'A0':
            p1a(0, 0)
        elif wk == 'B0':
            p1a(0, 1)
        elif wk[0] == 'a':
            p1a(int(wk[1:]))
        elif wk[0] == 'b':
            p1b(int(wk[1:]))
        elif wk == 'g':
            deadline(gate_ref)
        elif wk[0] == 'd':
            deadline(wcat[int(wk[1:])])
        elif wk == 'pq':
            prep_mat(ut0, wa_v, 0, 0)
        else:
            m = int(wk[1:])
            prep_mat(ut1 if m % 2 == 0 else ut0, wb_v, m * 512, m + 1)

    for waits, issues, work in SCHED:
        for n in waits:
            cps[n].wait()
        for n in issues:
            cps[n].start()
        for wk in work:
            do_work(wk)

    z = jnp.broadcast_to(jnp.sum(z_ref[...], axis=0, keepdims=True), (8, D))
    zc = _lane_perm([z[:, _cs(c)] for c in range(4)])
    for c in range(4):
        z_ref[:, _cs(c)] = zc[c]
        kb[0][c, 0:HALO, :] = jnp.zeros((HALO, 128), F32)
        vb[0][c, 0:HALO, :] = jnp.zeros((HALO, 128), F32)

    po_tasks = []
    for c in range(4):
        for q4 in range(4):
            po_tasks.append(lambda c=c, q4=q4: put_padded(
                tmp2_ref, c, wob_v[q4 * 128:(q4 + 1) * 128, _cs(c)].astype(F32), h0=8 * q4))
        for q4 in range(4):
            def t2(c=c, q4=q4):
                w2b[q4 * 64:(q4 + 1) * 64, _cs(c)] = _pk(gather_perm(tmp2_ref, c, 4 * q4, 4 * q4 + 4).astype(BF16))
            po_tasks.append(t2)
    for pi, (_, f) in enumerate(s1_pieces(0, 0, 0, HT)):
        if pi == 4:
            deadline(wcat[3])
        toks = f()
        for ti, tok in enumerate(toks[len(toks) // 2 - 1::len(toks) // 2]):
            tmp2_ref[0, pl.ds(pl.multiple_of(32 * ST + dz8, 8), 8), :] = tok
            po_tasks[2 * pi + ti]()

    step(0, TH, 0, None, 0, first=True, tailcyc=768)

    def pair_body(j, carry):
        i1 = 2 * j + 1
        r1 = pl.multiple_of(i1 * T, T)
        h2 = pl.multiple_of((i1 + 1) * TH, TH)
        step(pl.multiple_of(i1 * TH, TH), h2, r1, pl.multiple_of(r1 - T, T), 1)
        cp_o(i1 - 1).start()
        step(h2, pl.multiple_of((i1 + 2) * TH, TH), pl.multiple_of(r1 + T, T), r1, 0)
        cp_o(i1).start()
        return carry

    lax.fori_loop(0, (NT - 2) // 2, pair_body, 0)

    rl = (NT - 1) * T
    step((NT - 1) * TH, None, rl, rl - T, 1, tailcyc=0)
    cp_o(NT - 2).start()

    def cp_last(lo, cols, sem):
        return pltpu.make_async_copy(o_v.at[pl.ds(rl + lo, HT), cols], o_hbm.at[0, pl.ds(rl + lo, HT), cols],
                                     sem_o.at[sem])

    last = [cp_last(0, slice(0, D), NT - 1), cp_last(HT, slice(0, 384), NT), cp_last(HT, slice(384, D), NT + 1)]
    for _, f in s3_pieces(rl, 1, 0, HT):
        f()
    last[0].start()
    for n, (_, f) in enumerate(s3_pieces(rl, 1, HT, T)):
        f()
        if n >= 2:
            last[n - 1].start()
    for i in range(NT - 1):
        cp_o(i).wait()
    for c_ in last:
        c_.wait()


@jax.jit
def pallas_gated_mix__linear_attn_block__sliding_local_dilated__prompt_kernel(A_x, A_wqkv, A_wo, B_x, B_wqkv, B_wo, gate_w):
    anyspec = pl.BlockSpec(memory_space=pl.ANY)
    two = lambda shape, dt: [pltpu.VMEM(shape, dt)] * 2
    return pl.pallas_call(
        _kernel,
        grid=(1,),
        in_specs=[anyspec] * 7,
        out_specs=anyspec,
        out_shape=jax.ShapeDtypeStruct((1, S, D), BF16),
        scratch_shapes=[
            pltpu.SMEM((8,), jnp.int32),
            pltpu.VMEM((D,), BF16),
            pltpu.VMEM((S, D), BF16),
            pltpu.VMEM((D, 3 * D), BF16),
            pltpu.VMEM((D, D), BF16),
            pltpu.VMEM((D, 3 * D), BF16),
            pltpu.VMEM((D, D), BF16),
            pltpu.VMEM((S, D), BF16),
            pltpu.VMEM((S // 2 + 16, D), U32),
            pltpu.VMEM((D // 2, D), U32),
            *two((D // 2, D), U32), *two((D // 2, D), U32),
            *two((D // 2, D), U32),
            pltpu.VMEM((4, 64, 128), U32),
            pltpu.VMEM((D, D), F32),
            pltpu.VMEM((8, D), F32),
            pltpu.VMEM((4, 32 * ST + 16, 128), F32),
            pltpu.VMEM((4, 32 * ST + 16, 128), F32),
            *two((2, 32 * ST, 128), U32),
            pltpu.VMEM((S, 128), F32),
            pltpu.VMEM((S // 2, D), U32),
            *two((T, 2 * D), F32),
            *two((4, HALO + T, 128), F32),
            *two((4, HALO + T, 128), F32),
            *two((T // 2, 2 * D), U32),
            pltpu.VMEM((56, 128), F32),
            pltpu.SemaphoreType.DMA((NT,)),
            pltpu.SemaphoreType.DMA((11,)),
            pltpu.SemaphoreType.DMA((NT + 2,)),
        ],
        compiler_params=pltpu.CompilerParams(vmem_limit_bytes=100 * 1024 * 1024),
    )(A_x, A_wqkv, A_wo, B_wqkv, B_wo, gate_w, jnp.zeros((8,), jnp.int32))
```
